```python
import os as _os
_os.environ.setdefault("JAX_PLATFORMS", "cpu")
import jax
import jax.numpy as jnp

def _softmax(x, axis=-1):
    return jax.nn.softmax(x, axis=axis)
def _gelu(x):
    return jax.nn.gelu(x, approximate=True)
def _silu(x):
    return jax.nn.silu(x)
def _sigmoid(x):
    return jax.nn.sigmoid(x)
def _layernorm(x, axis=-1, eps=1e-5):
    m = jnp.mean(x, axis=axis, keepdims=True)
    v = jnp.var(x, axis=axis, keepdims=True)
    return (x - m) / jnp.sqrt(v + eps)
def _scatter_add(tgt, idx, src, axis=0):
    return tgt.at[idx].add(src)
def _segment_sum(src, seg, n):
    return jax.ops.segment_sum(src, seg, n)
class _Rng:
    def __init__(self, key):
        self._k = key
    def _next(self):
        self._k, sub = jax.random.split(self._k)
        return sub
    def normal(self, shape):
        return jax.random.normal(self._next(), shape, dtype=jnp.bfloat16)
    def randint(self, lo, hi, shape):
        return jax.random.randint(self._next(), shape, lo, hi, dtype=jnp.int32)
    def uniform(self, shape, lo=0.0, hi=1.0):
        return jax.random.uniform(self._next(), shape, jnp.bfloat16, lo, hi)
    def permutation(self, n):
        return jax.random.permutation(self._next(), n)


kernel_name = 'sequential_preLN__softmax_full_mha__swiglu_ffn__prompt'

def setup_inputs():
    _rng = _Rng(jax.random.key(int.from_bytes(__import__("os").urandom(4), "little")))
    _w = (lambda a: (lambda t: t.astype(jnp.bfloat16) if jnp.issubdtype(t.dtype, jnp.floating) else t)(jnp.asarray(a)))
    def _A_setup():
        B, S, D = 1, 2048, 512
        return {
            "x": _w((lambda *s: _rng.normal(s) * 0.05)(B, S, D)),
            "wqkv": _w((lambda *s: _rng.normal(s) * 0.05)(D, 3 * D)),
            "wo": _w((lambda *s: _rng.normal(s) * 0.05)(D, D)),
        }
    _A_in = _A_setup()

    def _B_setup():
        B, S, D, F = 1, 2048, 512, 1792
        return {
            "x": _w((lambda *s: _rng.normal(s) * 0.05)(B, S, D)),
            "w_gate": _w((lambda *s: _rng.normal(s) * 0.05)(D, F)),
            "w_up": _w((lambda *s: _rng.normal(s) * 0.05)(D, F)),
            "w_down": _w((lambda *s: _rng.normal(s) * 0.05)(F, D)),
        }
    _B_in = _B_setup()

    return {
        "A_x": _A_in["x"],
        "A_wqkv": _A_in["wqkv"],
        "A_wo": _A_in["wo"],
        "B_x": _B_in["x"],
        "B_w_gate": _B_in["w_gate"],
        "B_w_up": _B_in["w_up"],
        "B_w_down": _B_in["w_down"],
    }

def reference(A_x, A_wqkv, A_wo, B_x, B_w_gate, B_w_up, B_w_down):
    def _A_ref(x, wqkv, wo):
        B, S, D = x.shape
        H = 32; Dh = D // H
        qkv = (lambda x, *d: x.transpose(*d))((x @ wqkv).reshape(B, S, 3, H, Dh), 2, 0, 3, 1, 4)
        q, k, v = qkv[0], qkv[1], qkv[2]
        scale = Dh ** -0.5
        scores = jnp.einsum("bhqd,bhkd->bhqk", q, k) * scale
        p = _softmax(scores, axis=-1)
        o = jnp.einsum("bhqk,bhkd->bhqd", p, v)
        return (lambda x, *d: x.transpose(*d))(o, 0, 2, 1, 3).reshape(B, S, D) @ wo

    def _B_ref(x, w_gate, w_up, w_down):
        g = _silu(x @ w_gate)
        u = x @ w_up
        return (g * u) @ w_down

    x = A_x
    h = x + _A_ref(_layernorm(x, axis=-1), A_wqkv, A_wo)
    h2 = h + _B_ref(_layernorm(h, axis=-1), B_w_gate, B_w_up, B_w_down)
    return h2
```

```python
import math
import jax, jax.numpy as jnp
from jax import lax
from jax.experimental import pallas as pl
from jax.experimental.pallas import tpu as pltpu

S, D, H, DH, F = 2048, 512, 32, 16, 1792
TQ = 512
CK = 128
UNR = 4
PACE = 3
FC = 256
SKIP_ATT = 0
SKIP_FFN = 0
NC = S // CK
NQ = S // TQ
EPS = 1e-5
QSCALE = (DH ** -0.5) * math.log2(math.e)
bf16 = jnp.bfloat16
f32 = jnp.float32


def pk(x):
    return pltpu.bitcast(x, jnp.uint32)


def upk(x):
    return pltpu.bitcast(x, bf16)


def tree_reduce(x, op):
    n = x.shape[0] // 8
    parts = [x[8 * j:8 * (j + 1)] for j in range(n)]
    while len(parts) > 1:
        parts = [op(parts[2 * j], parts[2 * j + 1]) for j in range(len(parts) // 2)]
    return parts[0]


def _ln(x):
    mu = jnp.mean(x, axis=-1, keepdims=True)
    xc = x - mu
    var = jnp.mean(xc * xc, axis=-1, keepdims=True)
    return xc * lax.rsqrt(var + EPS)


def dot(a, b):
    return jnp.dot(a, b, preferred_element_type=f32)


def dot_nt(a, b):
    return lax.dot_general(a, b, (((1,), (1,)), ((), ())), preferred_element_type=f32)


def kernel(x_ref, wqkv_ref, wo_ref, wg_ref, wu_ref, wd_ref, o_ref,
           k_scr, qT_scr, vT_scr, wT_scr, qm_scr, sA, sB, m_scr, oT_scr, a_scr, z_ref):
    i = pl.program_id(0)

    def qk_chunk(c, g, qm, sdst):
        kc = upk(k_scr[g, c * CK // 2:(c + 1) * CK // 2, :])
        s = dot(kc, qm)
        sdst[0, c * CK:(c + 1) * CK, :] = s
        return tree_reduce(s, jnp.maximum)

    @pl.when(i == 0)
    def _():
        z_ref[0] = 0
        qm_scr[...] = jnp.zeros_like(qm_scr)
        wT_scr[0:D // 2, :] = pk(wqkv_ref[:, 0:D].astype(f32).T.astype(bf16))
        wT_scr[D // 2:D, :] = pk(wqkv_ref[:, 2 * D:3 * D].astype(f32).T.astype(bf16))

        def qkv_body(t, carry):
            r0 = pl.multiple_of(t * TQ, TQ)
            xn = _ln(x_ref[pl.ds(r0, TQ), :].astype(f32)).astype(bf16)
            kk = dot(xn, wqkv_ref[:, D:2 * D]).astype(bf16)
            for g in range(4):
                k_scr[g, pl.ds(pl.multiple_of(t * (TQ // 2), TQ // 2), TQ // 2), :] = pk(kk[:, g * 128:(g + 1) * 128])
            qv = dot_nt(upk(wT_scr[...]), xn)
            qT_scr[t] = pk((qv[0:D] * QSCALE).astype(bf16))
            vT_scr[t] = pk(qv[D:2 * D].astype(bf16))
            return carry
        lax.fori_loop(0, NQ, qkv_body, 0)

        qm_scr[0, 0:8, :] = qT_scr[0, 0:8, :]
        qm0 = upk(qm_scr[0])
        mx = jnp.full((8, TQ), -jnp.inf, f32)
        for c in range(NC):
            mx = jnp.maximum(mx, qk_chunk(c, 0, qm0, sA))
        m_scr[...] = jnp.broadcast_to(jnp.max(mx, axis=0, keepdims=True), (8, TQ))

    for h in range(1, H):
        qm_scr[h, (h % 8) * 8:(h % 8 + 1) * 8, :] = qT_scr[i, h * 8:(h + 1) * 8, :]
    qm_scr[H, 0:8, :] = qT_scr[jnp.minimum(i + 1, NQ - 1), 0:8, :]

    def one_head(h, m_cur, ssrc, sdst, z):
        hn = h + 1
        gn = lax.shift_right_logical(hn, 3) & 3
        qm = upk(qm_scr[hn])
        acc = jnp.zeros((DH, TQ), f32)
        lsum = jnp.zeros((8, TQ), f32)
        mx = jnp.full((8, TQ), -jnp.inf, f32)
        cm = []
        for c in range(NC):
            cmx = qk_chunk(c, gn, qm, sdst)
            cm.append(cmx)
            mx = jnp.maximum(mx, cmx)
            m_c = m_cur
            if PACE and c >= PACE:
                m_c = jnp.minimum(m_cur, jnp.maximum(m_cur, cm[c - PACE]))
            sv = ssrc[z, c * CK:(c + 1) * CK, :].reshape(CK // 8, 8, TQ)
            p = jnp.exp2(sv - m_c[None]).reshape(CK, TQ)
            lsum = lsum + tree_reduce(p, jnp.add)
            t, cc = divmod(c * CK, TQ)
            vt = upk(vT_scr[t, pl.ds(pl.multiple_of(h * 8, 8), 8), cc:cc + CK])
            acc = acc + dot(vt, p.astype(bf16))
        l = jnp.sum(lsum, axis=0, keepdims=True)
        oT_scr[pl.ds(pl.multiple_of(h * DH, DH), DH), :] = acc * (1.0 / l)
        return jnp.broadcast_to(jnp.max(mx, axis=0, keepdims=True), (8, TQ))

    def heads_body(j, m_cur):
        z = z_ref[0]
        for u in range(UNR):
            if u % 2 == 0:
                m_cur = one_head(UNR * j + u, m_cur, sA, sB, z)
            else:
                m_cur = one_head(UNR * j + u, m_cur, sB, sA, z)
        return m_cur
    if not SKIP_ATT:
        m_scr[...] = lax.fori_loop(0, H // UNR, heads_body, m_scr[...])
    else:
        oT_scr[...] = jnp.zeros_like(oT_scr)

    r0 = pl.multiple_of(i * TQ, TQ)
    o = oT_scr[...].T.astype(bf16)
    h1 = x_ref[pl.ds(r0, TQ), :].astype(f32) + dot(o, wo_ref[...])
    if SKIP_FFN:
        o_ref[...] = h1.astype(o_ref.dtype)
        return
    hn = _ln(h1).astype(bf16)
    for fc in range(F // FC):
        g = dot(hn, wg_ref[:, fc * FC:(fc + 1) * FC])
        u = dot(hn, wu_ref[:, fc * FC:(fc + 1) * FC])
        a = g * u * (0.5 * jnp.tanh(0.5 * g) + 0.5)
        a_scr[:, fc * FC:(fc + 1) * FC] = pk(a.astype(bf16))
    y = dot(upk(a_scr[...]), wd_ref[...])
    o_ref[...] = (h1 + y).astype(o_ref.dtype)


@jax.jit
def pallas_sequential_preLN__softmax_full_mha__swiglu_ffn__prompt_kernel(A_x, A_wqkv, A_wo, B_x, B_w_gate, B_w_up, B_w_down):
    x = A_x.reshape(S, D)
    full = lambda shape: pl.BlockSpec(shape, lambda i: (0,) * len(shape))
    out = pl.pallas_call(
        kernel,
        grid=(NQ,),
        in_specs=[full((S, D)), full((D, 3 * D)), full((D, D)), full((D, F)), full((D, F)), full((F, D))],
        out_specs=pl.BlockSpec((TQ, D), lambda i: (i, 0)),
        out_shape=jax.ShapeDtypeStruct((S, D), bf16),
        scratch_shapes=[
            pltpu.VMEM((4, S // 2, 128), jnp.uint32),
            pltpu.VMEM((NQ, D // 2, TQ), jnp.uint32),
            pltpu.VMEM((NQ, D // 2, TQ), jnp.uint32),
            pltpu.VMEM((D, D), jnp.uint32),
            pltpu.VMEM((H + 1, 64, TQ), jnp.uint32),
            pltpu.VMEM((1, S, TQ), f32),
            pltpu.VMEM((1, S, TQ), f32),
            pltpu.VMEM((8, TQ), f32),
            pltpu.VMEM((D, TQ), f32),
            pltpu.VMEM((TQ // 2, F), jnp.uint32),
            pltpu.SMEM((1,), jnp.int32),
        ],
        compiler_params=pltpu.CompilerParams(dimension_semantics=("arbitrary",),
                                             vmem_limit_bytes=100 * 1024 * 1024),
    )(x, A_wqkv, A_wo, B_w_gate, B_w_up, B_w_down)
    return out.reshape(1, S, D)
```

```python
import functools
import math

import jax
import jax.numpy as jnp
from jax import lax
from jax.experimental import pallas as pl
from jax.experimental.pallas import tpu as pltpu

S, D, H, DH, F = 2048, 512, 32, 16, 1792
TQ = 512
HW = TQ // 2
CK = 128
NC = S // CK
NQ = S // TQ
QB = 128
FB = 256
FC = 256
UNR_FAST = 8
UNR_SLOW = 2
SKEW_FAST, GATE_FAST = 3, -12
SKEW_SLOW, GATE_SLOW = 2, -12
LEVELS = (2, 4)
NT = 1 + 2 * len(LEVELS)
QROWS = -(-NT * DH // 32) * 32
EPS = 1e-5
QSCALE = (DH ** -0.5) * math.log2(math.e)
UNIT_MAX = 2.0 ** -9
RMAGIC = 12582912.0

bf16 = jnp.bfloat16
f32 = jnp.float32
u32 = jnp.uint32
i32 = jnp.int32
i8 = jnp.int8


def _pk(x):
    return pltpu.bitcast(x, u32)


def _upk(x):
    return pltpu.bitcast(x, bf16)


def _tree(x, op):
    parts = [x[8 * j:8 * (j + 1)] for j in range(x.shape[0] // 8)]
    while len(parts) > 1:
        parts = [op(parts[2 * j], parts[2 * j + 1]) for j in range(len(parts) // 2)]
    return parts[0]


def _allred8(m, op):
    for sh in (4, 2, 1):
        m = op(m, pltpu.roll(m, sh, 0))
    return m


def _after(x, dep):
    return jnp.minimum(x, jnp.maximum(x, dep))


def _after_rows(x, dep):
    dep = jnp.concatenate([dep] * (x.shape[1] // 128), axis=1)
    head = _after(pltpu.bitcast(x[0:8], i32), dep)
    return jnp.concatenate([pltpu.bitcast(head, u32), x[8:]], axis=0)


def _ln(x):
    mu = jnp.mean(x, axis=-1, keepdims=True)
    xc = x - mu
    var = jnp.mean(xc * xc, axis=-1, keepdims=True)
    return xc * lax.rsqrt(var + EPS)


def _dot(a, b):
    return jnp.dot(a, b, preferred_element_type=f32)


def _dot_nt(a, b):
    return lax.dot_general(a, b, (((1,), (1,)), ((), ())), preferred_element_type=f32)


def _rbits(v, a):
    return pltpu.bitcast(v + RMAGIC * 2.0 ** -a, i32)


def _limbs(x):
    prev, a_prev = _rbits(x, 0), 0
    main, fine, coarse = prev, [], []
    for a in LEVELS:
        r = _rbits(x, a)
        fine.append(r - (prev << (a - a_prev)))
        coarse.append(_rbits(x, -a))
        prev, a_prev = r, a
    return main, fine, coarse


def _kernel(x_hbm, wqkv_hbm, wo_hbm, wg_hbm, wu_hbm, wd_hbm, o_ref,
            x_ref, wqkv_ref, wo_ref, wg_ref, wu_ref, wd_ref, sems,
            wT_scr, xp_scr, xn_scr, xf_scr, kT_scr, kmax_scr, k8_scr, q8_scr, b_scr, vT_scr,
            k_scr, qT_scr, s_a, s_b, m_scr, oT_scr, a_scr, flag_ref):
    i = pl.program_id(0)

    def x_copy(t):
        rows = pl.ds(t * TQ, TQ)
        return pltpu.make_async_copy(x_hbm.at[rows, :], x_ref.at[rows, :], sems.at[t])

    def wqkv_copy(j):
        cols = pl.ds(j * D, D)
        return pltpu.make_async_copy(wqkv_hbm.at[:, cols], wqkv_ref.at[:, cols], sems.at[NQ + j])

    def w_copies():
        pairs = ((wo_hbm, wo_ref), (wg_hbm, wg_ref), (wu_hbm, wu_ref), (wd_hbm, wd_ref))
        return [pltpu.make_async_copy(s, d, sems.at[NQ + 3 + j]) for j, (s, d) in enumerate(pairs)]

    def half_rows(start, n):
        return pl.ds(pl.multiple_of(start // 2, n // 2), n // 2)

    def transposed_weight(j):
        return _pk(wqkv_ref[:, j * D:(j + 1) * D].astype(f32).T.astype(bf16))


    def fast_weights(tile, h):
        w = jnp.concatenate([q8_scr[tile, h], jnp.zeros(((128 - QROWS) // 4, TQ), u32)], axis=0)
        return pltpu.bitcast(w, i8)

    def fast_scores(kc, qm, bv):
        v = jnp.dot(pltpu.bitcast(kc, i8), qm, preferred_element_type=i32)
        n = v.shape[1]
        return pltpu.bitcast((bv[None] - v.reshape(CK // 8, 8, n)).reshape(CK, n), f32)

    def slow_weights(tile, h):
        g8 = pl.multiple_of(lax.shift_right_logical(h, 3) * 64, 64)
        nb = TQ // QB
        qg = jnp.concatenate([qT_scr[tile * nb + b, pl.ds(g8, 64), :] for b in range(nb)], axis=1)
        row = lax.shift_right_logical(lax.broadcasted_iota(i32, (64, TQ), 0), 3)
        return _upk(jnp.where(row == (h & 7), qg, jnp.zeros_like(qg)))

    @pl.when(i == 0)
    def _():
        wqkv_copy(1).start()
        x_copy(0).start()
        flag_ref[0] = 0
        kmax_scr[...] = jnp.zeros_like(kmax_scr)
        ones_row = jnp.where(lax.broadcasted_iota(i32, (8, TQ), 0) == 0,
                             jnp.uint32(0x3F80), jnp.uint32(0))
        for t in range(NQ):
            for h in range(H):
                vT_scr[t, h, 8:16, :] = ones_row
        wqkv_copy(1).wait()
        for t in range(1, NQ):
            x_copy(t).start()
        wqkv_copy(0).start()
        wqkv_copy(2).start()
        wT_scr[0:D // 2, :] = transposed_weight(1)

        for t in range(NQ):
            if t == 0:
                x_copy(0).wait()
            if t == 1:
                x_copy(1).wait()
                x_copy(2).wait()
            if t == 3:
                x_copy(3).wait()
                wqkv_copy(0).wait()
                wqkv_copy(2).wait()
                for cp in w_copies():
                    cp.start()
            for b in range(TQ // QB):
                r0 = t * TQ + b * QB
                xn = _ln(x_ref[r0:r0 + QB, :].astype(f32))
                for g in range(4):
                    xf_scr[t % 2, g, pl.ds(b, QB, stride=4), :] = xn[:, g * 128:(g + 1) * 128]
                xn = xn.astype(bf16)
                xn_scr[r0 // 2:(r0 + QB) // 2, :] = _pk(xn)
                kt = _dot_nt(_upk(wT_scr[0:D // 2, :]), xn)
                kT_scr[t, :, b * QB:(b + 1) * QB] = kt
                ka = jnp.abs(kt).reshape(H, 2, 8, QB)
                kmax_scr[...] = jnp.maximum(kmax_scr[...], jnp.maximum(ka[:, 0], ka[:, 1]))
            for b in range(TQ // QB):
                r0 = t * TQ + b * QB
                xp = jnp.concatenate([xf_scr[t % 2, g, b * QB:(b + 1) * QB, :] for g in range(4)], axis=1)
                xp_scr[r0 // 2:(r0 + QB) // 2, :] = _pk(xp.astype(bf16))
        wT_scr[D // 2:D, :] = transposed_weight(0)
        wT_scr[D:3 * D // 2, :] = transposed_weight(2)

        km = jnp.max(kmax_scr[...], axis=2, keepdims=True)
        km = jnp.maximum(jnp.max(km, axis=1, keepdims=True), 1e-30)
        kmax_scr[...] = jnp.broadcast_to(km, (H, 8, 128))

        def quant_k(t, h):
            kinv = jnp.concatenate([127.0 / kmax_scr[h]] * 4, axis=1)
            y = kT_scr[t, h * DH:(h + 1) * DH, :]
            y = (y.reshape(2, 8, TQ) * kinv[None]).reshape(DH, TQ)
            main, fine, coarse = _limbs(y)
            words = [((v[:, 0:128] & 0xFF) | ((v[:, 128:256] & 0xFF) << 8)
                      | ((v[:, 256:384] & 0xFF) << 16) | (v[:, 384:512] << 24))
                     for v in [main] + coarse + fine]
            words.append(jnp.zeros((128 - NT * DH, 128), i32))
            wt = jnp.concatenate(words, axis=0).T
            k8_scr[h, pl.ds(pl.multiple_of(t * 128, 128), 128), :] = pltpu.bitcast(wt, u32)
            return wt[120:128]

        def body_b(t, umax):
            for b in range(TQ // QB):
                rows = half_rows(t * TQ + b * QB, QB)
                qt = _dot_nt(_upk(wT_scr[D // 2:D, :]), _upk(xn_scr[rows, :]))
                dep = functools.reduce(jnp.bitwise_or, [quant_k(t, h) for h in range(b * 8, b * 8 + 8)])
                for h in range(H):
                    q = qt[h * DH:(h + 1) * DH]
                    kmx = kmax_scr[h]
                    qa = jnp.abs(q)
                    qmx = _allred8(jnp.maximum(qa[0:8], qa[8:16]), jnp.maximum)
                    uraw = jnp.maximum(qmx * kmx * (QSCALE / (127.0 * 127.0)), 2.0 ** -60)
                    umax = jnp.maximum(umax, uraw)
                    ub = (pltpu.bitcast(uraw, i32) + 0x7FFFFF) & 0x7F800000
                    b_scr[t, h, :, b * QB:(b + 1) * QB] = ub + ((23 << 23) + (1 << 22))
                    sc = kmx * pltpu.bitcast((254 << 23) - ub, f32) * (QSCALE / 127.0)
                    main, fine, coarse = _limbs((q.reshape(2, 8, QB) * sc[None]).reshape(DH, QB))
                    limbs = [main] + fine + coarse + [jnp.zeros((QROWS - NT * DH, QB), i32)]
                    q8_scr[t, h, :, b * QB:(b + 1) * QB] = _pk(jnp.concatenate(limbs, axis=0).astype(i8))
                xp = _upk(_after_rows(xp_scr[rows, :], dep))
                vb = _pk(_dot_nt(_upk(wT_scr[D:3 * D // 2, :]), xp).astype(bf16))
                for h in range(H):
                    vT_scr[t, h, 0:8, b * QB:(b + 1) * QB] = vb[h * 8:(h + 1) * 8]
            return umax
        umax = lax.fori_loop(0, NQ, body_b, jnp.zeros((8, QB), f32))
        flag_ref[1] = jnp.where(jnp.max(umax) <= UNIT_MAX, 1, 0).astype(i32)

        @pl.when(flag_ref[1] == 1)
        def _():
            qm, bv, mx = fast_weights(0, 0), b_scr[0, 0], None
            for c in range(NC):
                s = fast_scores(k8_scr[0, c * CK // 4:(c + 1) * CK // 4, :], qm, bv)
                s_a[0, c * CK:(c + 1) * CK, :] = s
                cm = _tree(s, jnp.minimum)
                mx = cm if mx is None else jnp.minimum(mx, cm)
            m_scr[...] = _allred8(mx, jnp.minimum)

        @pl.when(flag_ref[1] == 0)
        def _():
            def body_s(t, carry):
                rows = half_rows(t * QB, QB)
                kk = _dot(_upk(xp_scr[rows, :]), wqkv_ref[:, D:2 * D]).astype(bf16)
                for g in range(4):
                    k_scr[g, rows, :] = _pk(kk[:, g * 128:(g + 1) * 128])
                qq = _dot_nt(_upk(wT_scr[D // 2:D, :]), _upk(xn_scr[rows, :]))
                qT_scr[t] = _pk((qq * QSCALE).astype(bf16))
                return carry
            lax.fori_loop(0, S // QB, body_s, 0)
            qm = slow_weights(0, 0)

            def body_p(c, mx):
                s = -_dot(_upk(k_scr[0, half_rows(c * CK, CK), :]), qm)
                s_a[0, pl.ds(pl.multiple_of(c * CK, CK), CK), :] = s
                return jnp.minimum(mx, _tree(s, jnp.minimum))
            mx = lax.fori_loop(0, NC, body_p, jnp.full((8, TQ), jnp.inf, f32))
            m_scr[...] = _allred8(mx, jnp.minimum)

    def next_head(h):
        hn = (h + 1) & (H - 1)
        tn = jnp.minimum(i + lax.shift_right_logical(h + 1, 5), NQ - 1)
        return hn, tn

    def softmax_pv(h, c, m, src, z, cols):
        n = cols.stop - cols.start
        sv = src[z, c * CK:(c + 1) * CK, cols].reshape(CK // 8, 8, n)
        p = jnp.exp2(m[None] - sv).reshape(CK, n)
        t, cc = divmod(c * CK, TQ)
        return p, t, cc

    def fast_head(h, m_cur, src, dst, z):
        hn, tn = next_head(h)
        qm, bv = fast_weights(tn, hn), b_scr[tn, hn]
        cols = [slice(s * HW, (s + 1) * HW) for s in range(2)]
        st = [dict(mx=None, acc=None, ss=[], m=m_cur[:, cols[s]]) for s in range(2)]

        def qk(s, c):
            kc = k8_scr[hn, c * CK // 4:(c + 1) * CK // 4, :]
            if s == 1 and c >= 1:
                kc = _after_rows(kc, pltpu.bitcast(st[0]["ss"][c - 1][0:8, 0:128], i32))
            v = fast_scores(kc, qm[:, cols[s]], bv[:, cols[s]])
            dst[0, c * CK:(c + 1) * CK, cols[s]] = v
            d = st[s]
            d["ss"].append(v)
            cm = _tree(v, jnp.minimum)
            d["mx"] = cm if d["mx"] is None else jnp.minimum(d["mx"], cm)

        for c in range(SKEW_FAST):
            for s in range(2):
                qk(s, c)
        for c in range(NC):
            for s in range(2):
                d = st[s]
                if c >= 1:
                    gc, gr = divmod(c * 16 + GATE_FAST, 16)
                    dep = d["ss"][gc][gr * 8:(gr + 1) * 8, 128:256]
                    d["m"] = _after(d["m"], jnp.concatenate([dep] * 2, axis=1))
                p, t, cc = softmax_pv(h, c, d["m"], src, z, cols[s])
                pv = _dot(_upk(vT_scr[t, h, :, cc:cc + CK]), p.astype(bf16))[0:24]
                d["acc"] = pv if d["acc"] is None else d["acc"] + pv
            if c + SKEW_FAST < NC:
                for s in range(2):
                    qk(s, c + SKEW_FAST)
        acc = jnp.concatenate([st[0]["acc"], st[1]["acc"]], axis=1)
        oT_scr[pl.ds(pl.multiple_of(h * DH, DH), DH), :] = acc[0:16] * (1.0 / acc[16:17])
        return _allred8(jnp.concatenate([st[0]["mx"], st[1]["mx"]], axis=1), jnp.minimum)

    def slow_head(h, m_cur, src, dst, z):
        hn, tn = next_head(h)
        gn = lax.shift_right_logical(hn, 3)
        qm = slow_weights(tn, hn)
        acc = lsum = mx = None
        ss = []

        def qk(c):
            nonlocal mx
            s = -_dot(_upk(k_scr[gn, c * CK // 2:(c + 1) * CK // 2, :]), qm)
            dst[0, c * CK:(c + 1) * CK, :] = s
            ss.append(s)
            cm = _tree(s, jnp.minimum)
            mx = cm if mx is None else jnp.minimum(mx, cm)

        for c in range(SKEW_SLOW):
            qk(c)
        m = m_cur
        for c in range(NC):
            if c >= 1:
                gc, gr = divmod(c * 16 + GATE_SLOW, 16)
                m = _after(m, jnp.concatenate([ss[gc][gr * 8:(gr + 1) * 8, 384:512]] * 4, axis=1))
            p, t, cc = softmax_pv(h, c, m, src, z, slice(0, TQ))
            ls = _tree(p, jnp.add)
            lsum = ls if lsum is None else lsum + ls
            pv = _dot(_upk(vT_scr[t, h, 0:8, cc:cc + CK]), p.astype(bf16))
            acc = pv if acc is None else acc + pv
            if c + SKEW_SLOW < NC:
                qk(c + SKEW_SLOW)
        l = jnp.sum(lsum, axis=0, keepdims=True)
        oT_scr[pl.ds(pl.multiple_of(h * DH, DH), DH), :] = acc * (1.0 / l)
        return _allred8(mx, jnp.minimum)

    def heads_loop(head_fn, unroll):
        def body(j, m):
            z = flag_ref[0]
            for u in range(unroll):
                src, dst = (s_a, s_b) if u % 2 == 0 else (s_b, s_a)
                m = head_fn(j * unroll + u, m, src, dst, z)
            return m
        m_scr[...] = lax.fori_loop(0, H // unroll, body, m_scr[...])

    @pl.when(flag_ref[1] == 1)
    def _():
        heads_loop(fast_head, UNR_FAST)

    @pl.when(flag_ref[1] == 0)
    def _():
        heads_loop(slow_head, UNR_SLOW)

    @pl.when(i == 0)
    def _():
        for cp in w_copies():
            cp.wait()

    h1s, hns = [], []
    for b in range(TQ // FB):
        r0 = pl.multiple_of(i * TQ + b * FB, FB)
        o = oT_scr[:, b * FB:(b + 1) * FB].T.astype(bf16)
        h1 = x_ref[pl.ds(r0, FB), :].astype(f32) + _dot(o, wo_ref[...])
        h1s.append(h1)
        hns.append(_ln(h1).astype(bf16))
    for b in range(TQ // FB):
        rows = slice(b * FB // 2, (b + 1) * FB // 2)
        for fc in range(F // FC):
            g = _dot(hns[b], wg_ref[:, fc * FC:(fc + 1) * FC])
            u = _dot(hns[b], wu_ref[:, fc * FC:(fc + 1) * FC])
            a = g * u * (0.5 * jnp.tanh(0.5 * g) + 0.5)
            a_scr[rows, fc * FC:(fc + 1) * FC] = _pk(a.astype(bf16))
        y = _dot(_upk(a_scr[rows, :]), wd_ref[...])
        o_ref[b * FB:(b + 1) * FB, :] = (h1s[b] + y).astype(o_ref.dtype)


@jax.jit
def pallas_sequential_preLN__softmax_full_mha__swiglu_ffn__prompt_kernel(
    A_x: jax.Array,
    A_wqkv: jax.Array,
    A_wo: jax.Array,
    B_x: jax.Array,
    B_w_gate: jax.Array,
    B_w_up: jax.Array,
    B_w_down: jax.Array,
):
    del B_x
    out = pl.pallas_call(
        _kernel,
        grid=(NQ,),
        in_specs=[pl.BlockSpec(memory_space=pl.ANY)] * 6,
        out_specs=pl.BlockSpec((TQ, D), lambda i: (i, 0)),
        out_shape=jax.ShapeDtypeStruct((S, D), bf16),
        scratch_shapes=[
            pltpu.VMEM((S, D), bf16),
            pltpu.VMEM((D, 3 * D), bf16),
            pltpu.VMEM((D, D), bf16),
            pltpu.VMEM((D, F), bf16),
            pltpu.VMEM((D, F), bf16),
            pltpu.VMEM((F, D), bf16),
            pltpu.SemaphoreType.DMA((NQ + 7,)),
            pltpu.VMEM((3 * D // 2, D), u32),
            pltpu.VMEM((S // 2, D), u32),
            pltpu.VMEM((S // 2, D), u32),
            pltpu.VMEM((2, 4, TQ, 128), f32),
            pltpu.VMEM((NQ, D, TQ), f32),
            pltpu.VMEM((H, 8, 128), f32),
            pltpu.VMEM((H, S // 4, 128), u32),
            pltpu.VMEM((NQ, H, QROWS // 4, TQ), u32),
            pltpu.VMEM((NQ, H, 8, TQ), i32),
            pltpu.VMEM((NQ, H, 16, TQ), u32),
            pltpu.VMEM((4, S // 2, 128), u32),
            pltpu.VMEM((S // QB, D // 2, QB), u32),
            pltpu.VMEM((1, S, TQ), f32),
            pltpu.VMEM((1, S, TQ), f32),
            pltpu.VMEM((8, TQ), f32),
            pltpu.VMEM((D, TQ), f32),
            pltpu.VMEM((TQ // 2, F), u32),
            pltpu.SMEM((2,), i32),
        ],
        compiler_params=pltpu.CompilerParams(
            dimension_semantics=("arbitrary",),
            vmem_limit_bytes=110 * 1024 * 1024,
        ),
    )(A_x.reshape(S, D), A_wqkv, A_wo, B_w_gate, B_w_up, B_w_down)
    return out.reshape(1, S, D)
```

```python
import functools
import math

import jax
import jax.numpy as jnp
from jax import lax
from jax.experimental import pallas as pl
from jax.experimental.pallas import tpu as pltpu

S, D, H, DH, F = 2048, 512, 32, 16, 1792
TQ = 512
HW = TQ // 2
CK = 128
NC = S // CK
NQ = S // TQ
QB = 128
FR = 128
UNR_FAST = H * FR // TQ
UNR_SLOW = 2
SKEW_SOLO, GATE_SOLO = 3, -12
SKEW_FUSE, GATE_FUSE = 2, -52
SKEW_SLOW, GATE_SLOW = 2, -12
LEVELS = (2, 4)
NT = 1 + 2 * len(LEVELS)
QROWS = -(-NT * DH // 32) * 32
EPS = 1e-5
QSCALE = (DH ** -0.5) * math.log2(math.e)
UNIT_MAX = 2.0 ** -9
RMAGIC = 12582912.0

bf16 = jnp.bfloat16
f32 = jnp.float32
u32 = jnp.uint32
i32 = jnp.int32
i8 = jnp.int8


def _pk(x):
    return pltpu.bitcast(x, u32)


def _upk(x):
    return pltpu.bitcast(x, bf16)


def _tree(x, op):
    parts = [x[8 * j:8 * (j + 1)] for j in range(x.shape[0] // 8)]
    while len(parts) > 1:
        parts = [op(parts[2 * j], parts[2 * j + 1]) for j in range(len(parts) // 2)]
    return parts[0]


def _allred8(m, op):
    for sh in (4, 2, 1):
        m = op(m, pltpu.roll(m, sh, 0))
    return m


def _after(x, dep):
    return jnp.minimum(x, jnp.maximum(x, dep))


def _after_rows(x, dep):
    dep = jnp.concatenate([dep] * (x.shape[1] // 128), axis=1)
    head = _after(pltpu.bitcast(x[0:8], i32), dep)
    return jnp.concatenate([pltpu.bitcast(head, u32), x[8:]], axis=0)


def _ln(x):
    mu = jnp.mean(x, axis=-1, keepdims=True)
    xc = x - mu
    var = jnp.mean(xc * xc, axis=-1, keepdims=True)
    return xc * lax.rsqrt(var + EPS)


def _dot(a, b):
    return jnp.dot(a, b, preferred_element_type=f32)


def _dot_nt(a, b):
    return lax.dot_general(a, b, (((1,), (1,)), ((), ())), preferred_element_type=f32)


def _rbits(v, a):
    return pltpu.bitcast(v + RMAGIC * 2.0 ** -a, i32)


def _limbs(x):
    prev, a_prev = _rbits(x, 0), 0
    main, fine, coarse = prev, [], []
    for a in LEVELS:
        r = _rbits(x, a)
        fine.append(r - (prev << (a - a_prev)))
        coarse.append(_rbits(x, -a))
        prev, a_prev = r, a
    return main, fine, coarse


def _kernel(x_hbm, wqkv_hbm, wo_hbm, wg_hbm, wu_hbm, wd_hbm, o_ref,
            x_ref, wqkv_ref, wo_ref, wg_ref, wu_ref, wd_ref, sems,
            wT_scr, xp_scr, xn_scr, xf_scr, kT_scr, kmax_scr, k8_scr, q8_scr, b_scr, vT_scr,
            k_scr, qT_scr, s_a, s_b, m_scr, oT_scr, h1_scr, hn_scr, a_scr, flag_ref):
    i = pl.program_id(0)

    def x_copy(t):
        rows = pl.ds(t * TQ, TQ)
        return pltpu.make_async_copy(x_hbm.at[rows, :], x_ref.at[rows, :], sems.at[t])

    def wqkv_copy(j):
        cols = pl.ds(j * D, D)
        return pltpu.make_async_copy(wqkv_hbm.at[:, cols], wqkv_ref.at[:, cols], sems.at[NQ + j])

    def w_copies():
        pairs = ((wo_hbm, wo_ref), (wg_hbm, wg_ref), (wu_hbm, wu_ref), (wd_hbm, wd_ref))
        return [pltpu.make_async_copy(s, d, sems.at[NQ + 3 + j]) for j, (s, d) in enumerate(pairs)]

    def half_rows(start, n):
        return pl.ds(pl.multiple_of(start // 2, n // 2), n // 2)

    def transposed_weight(j):
        return _pk(wqkv_ref[:, j * D:(j + 1) * D].astype(f32).T.astype(bf16))


    def fast_weights(tile, h):
        w = jnp.concatenate([q8_scr[tile, h], jnp.zeros(((128 - QROWS) // 4, TQ), u32)], axis=0)
        return pltpu.bitcast(w, i8)

    def fast_scores(kc, qm, bv):
        v = jnp.dot(pltpu.bitcast(kc, i8), qm, preferred_element_type=i32)
        n = v.shape[1]
        return pltpu.bitcast((bv[None] - v.reshape(CK // 8, 8, n)).reshape(CK, n), f32)

    def slow_weights(tile, h):
        g8 = pl.multiple_of(lax.shift_right_logical(h, 3) * 64, 64)
        nb = TQ // QB
        qg = jnp.concatenate([qT_scr[tile * nb + b, pl.ds(g8, 64), :] for b in range(nb)], axis=1)
        row = lax.shift_right_logical(lax.broadcasted_iota(i32, (64, TQ), 0), 3)
        return _upk(jnp.where(row == (h & 7), qg, jnp.zeros_like(qg)))

    @pl.when(i == 0)
    def _():
        wqkv_copy(1).start()
        x_copy(0).start()
        flag_ref[0] = 0
        kmax_scr[...] = jnp.zeros_like(kmax_scr)
        ones_row = jnp.where(lax.broadcasted_iota(i32, (8, TQ), 0) == 0,
                             jnp.uint32(0x3F80), jnp.uint32(0))
        for t in range(NQ):
            for h in range(H):
                vT_scr[t, h, 8:16, :] = ones_row
        wqkv_copy(1).wait()
        x_copy(0).wait()
        for t in range(1, NQ):
            x_copy(t).start()
        wqkv_copy(0).start()
        wqkv_copy(2).start()
        wT_scr[0:D // 2, :] = transposed_weight(1)

        for t in range(NQ):
            if t == 1:
                x_copy(1).wait()
                x_copy(2).wait()
            if t == 3:
                x_copy(3).wait()
                wqkv_copy(0).wait()
                wqkv_copy(2).wait()
                for cp in w_copies():
                    cp.start()
            for b in range(TQ // QB):
                r0 = t * TQ + b * QB
                xn = _ln(x_ref[r0:r0 + QB, :].astype(f32))
                for g in range(4):
                    xf_scr[t % 2, g, pl.ds(b, QB, stride=4), :] = xn[:, g * 128:(g + 1) * 128]
                xn = xn.astype(bf16)
                xn_scr[r0 // 2:(r0 + QB) // 2, :] = _pk(xn)
                kt = _dot_nt(_upk(wT_scr[0:D // 2, :]), xn)
                kT_scr[t, :, b * QB:(b + 1) * QB] = kt
                ka = jnp.abs(kt).reshape(H, 2, 8, QB)
                kmax_scr[...] = jnp.maximum(kmax_scr[...], jnp.maximum(ka[:, 0], ka[:, 1]))
            for b in range(TQ // QB):
                r0 = t * TQ + b * QB
                xp = jnp.concatenate([xf_scr[t % 2, g, b * QB:(b + 1) * QB, :] for g in range(4)], axis=1)
                xp_scr[r0 // 2:(r0 + QB) // 2, :] = _pk(xp.astype(bf16))
        wT_scr[D // 2:D, :] = transposed_weight(0)
        wT_scr[D:3 * D // 2, :] = transposed_weight(2)

        km = jnp.max(kmax_scr[...], axis=2, keepdims=True)
        km = jnp.maximum(jnp.max(km, axis=1, keepdims=True), 1e-30)
        kmax_scr[...] = jnp.broadcast_to(km, (H, 8, 128))

        def quant_k(t, h):
            kinv = jnp.concatenate([127.0 / kmax_scr[h]] * 4, axis=1)
            y = kT_scr[t, h * DH:(h + 1) * DH, :]
            y = (y.reshape(2, 8, TQ) * kinv[None]).reshape(DH, TQ)
            main, fine, coarse = _limbs(y)
            words = [((v[:, 0:128] & 0xFF) | ((v[:, 128:256] & 0xFF) << 8)
                      | ((v[:, 256:384] & 0xFF) << 16) | (v[:, 384:512] << 24))
                     for v in [main] + coarse + fine]
            words.append(jnp.zeros((128 - NT * DH, 128), i32))
            wt = jnp.concatenate(words, axis=0).T
            k8_scr[h, pl.ds(pl.multiple_of(t * 128, 128), 128), :] = pltpu.bitcast(wt, u32)
            return wt[120:128]

        def body_b(t, umax):
            for b in range(TQ // QB):
                rows = half_rows(t * TQ + b * QB, QB)
                qt = _dot_nt(_upk(wT_scr[D // 2:D, :]), _upk(xn_scr[rows, :]))
                dep = functools.reduce(jnp.bitwise_or, [quant_k(t, h) for h in range(b * 8, b * 8 + 8)])
                for h in range(H):
                    q = qt[h * DH:(h + 1) * DH]
                    kmx = kmax_scr[h]
                    qa = jnp.abs(q)
                    qmx = _allred8(jnp.maximum(qa[0:8], qa[8:16]), jnp.maximum)
                    uraw = jnp.maximum(qmx * kmx * (QSCALE / (127.0 * 127.0)), 2.0 ** -60)
                    umax = jnp.maximum(umax, uraw)
                    ub = (pltpu.bitcast(uraw, i32) + 0x7FFFFF) & 0x7F800000
                    b_scr[t, h, :, b * QB:(b + 1) * QB] = ub + ((23 << 23) + (1 << 22))
                    sc = kmx * pltpu.bitcast((254 << 23) - ub, f32) * (QSCALE / 127.0)
                    main, fine, coarse = _limbs((q.reshape(2, 8, QB) * sc[None]).reshape(DH, QB))
                    limbs = [main] + fine + coarse + [jnp.zeros((QROWS - NT * DH, QB), i32)]
                    q8_scr[t, h, :, b * QB:(b + 1) * QB] = _pk(jnp.concatenate(limbs, axis=0).astype(i8))
                xp = _upk(_after_rows(xp_scr[rows, :], dep))
                vb = _pk(_dot_nt(_upk(wT_scr[D:3 * D // 2, :]), xp).astype(bf16))
                for h in range(H):
                    vT_scr[t, h, 0:8, b * QB:(b + 1) * QB] = vb[h * 8:(h + 1) * 8]
            return umax
        umax = lax.fori_loop(0, NQ, body_b, jnp.zeros((8, QB), f32))
        flag_ref[1] = jnp.where(jnp.max(umax) <= UNIT_MAX, 1, 0).astype(i32)

        @pl.when(flag_ref[1] == 1)
        def _():
            qm, bv, mx = fast_weights(0, 0), b_scr[0, 0], None
            for c in range(NC):
                s = fast_scores(k8_scr[0, c * CK // 4:(c + 1) * CK // 4, :], qm, bv)
                s_a[0, c * CK:(c + 1) * CK, :] = s
                cm = _tree(s, jnp.minimum)
                mx = cm if mx is None else jnp.minimum(mx, cm)
            m_scr[...] = _allred8(mx, jnp.minimum)

        @pl.when(flag_ref[1] == 0)
        def _():
            def body_s(t, carry):
                rows = half_rows(t * QB, QB)
                kk = _dot(_upk(xp_scr[rows, :]), wqkv_ref[:, D:2 * D]).astype(bf16)
                for g in range(4):
                    k_scr[g, rows, :] = _pk(kk[:, g * 128:(g + 1) * 128])
                qq = _dot_nt(_upk(wT_scr[D // 2:D, :]), _upk(xn_scr[rows, :]))
                qT_scr[t] = _pk((qq * QSCALE).astype(bf16))
                return carry
            lax.fori_loop(0, S // QB, body_s, 0)
            qm = slow_weights(0, 0)

            def body_p(c, mx):
                s = -_dot(_upk(k_scr[0, half_rows(c * CK, CK), :]), qm)
                s_a[0, pl.ds(pl.multiple_of(c * CK, CK), CK), :] = s
                return jnp.minimum(mx, _tree(s, jnp.minimum))
            mx = lax.fori_loop(0, NC, body_p, jnp.full((8, TQ), jnp.inf, f32))
            m_scr[...] = _allred8(mx, jnp.minimum)

    def next_head(h):
        hn = (h + 1) & (H - 1)
        tn = jnp.minimum(i + lax.shift_right_logical(h + 1, 5), NQ - 1)
        return hn, tn

    def probs(c, m, src, z, cols):
        n = cols.stop - cols.start
        sv = src[z, c * CK:(c + 1) * CK, cols].reshape(CK // 8, 8, n)
        return jnp.exp2(m[None] - sv).reshape(CK, n)

    def v_rows(h, c, with_ones):
        t, cc = divmod(c * CK, TQ)
        return _upk(vT_scr[t, h, 0:(16 if with_ones else 8), cc:cc + CK])

    def fast_head(h, m_cur, src, dst, z, hook=None):
        solo = hook is None
        skew, gate = (SKEW_SOLO, GATE_SOLO) if solo else (SKEW_FUSE, GATE_FUSE)
        hn, tn = next_head(h)
        qm, bv = fast_weights(tn, hn), b_scr[tn, hn]
        cols = [slice(s * HW, (s + 1) * HW) for s in range(2)]
        st = [dict(mx=None, acc=None, ss=[], m=m_cur[:, cols[s]]) for s in range(2)]

        def qk(s, c):
            kc = k8_scr[hn, c * CK // 4:(c + 1) * CK // 4, :]
            if solo and s == 1 and c >= 1:
                kc = _after_rows(kc, pltpu.bitcast(st[0]["ss"][c - 1][0:8, 0:128], i32))
            v = fast_scores(kc, qm[:, cols[s]], bv[:, cols[s]])
            dst[0, c * CK:(c + 1) * CK, cols[s]] = v
            d = st[s]
            d["ss"].append(v)
            cm = _tree(v, jnp.minimum)
            d["mx"] = cm if d["mx"] is None else jnp.minimum(d["mx"], cm)

        for c in range(skew):
            for s in range(2):
                qk(s, c)
        for c in range(NC):
            for s in range(2):
                d = st[s]
                gc, gr = divmod(c * 16 + gate, 16)
                if gc >= 0:
                    dep = d["ss"][gc][gr * 8:(gr + 1) * 8, 128:256]
                    d["m"] = _after(d["m"], jnp.concatenate([dep] * 2, axis=1))
                p = probs(c, d["m"], src, z, cols[s])
                pv = _dot(v_rows(h, c, solo), p.astype(bf16))
                pv = pv[0:24] if solo else jnp.concatenate([pv, _tree(p, jnp.add)], axis=0)
                d["acc"] = pv if d["acc"] is None else d["acc"] + pv
            for s in range(2):
                if not solo:
                    hook(2 * c + s)
                if c + skew < NC:
                    qk(s, c + skew)
        acc = jnp.concatenate([st[0]["acc"], st[1]["acc"]], axis=1)
        l = acc[16:17] if solo else jnp.sum(acc[16:24], axis=0, keepdims=True)
        oT_scr[pl.ds(pl.multiple_of(h * DH, DH), DH), :] = acc[0:16] * (1.0 / l)
        return _allred8(jnp.concatenate([st[0]["mx"], st[1]["mx"]], axis=1), jnp.minimum)

    def slow_head(h, m_cur, src, dst, z):
        hn, tn = next_head(h)
        gn = lax.shift_right_logical(hn, 3)
        qm = slow_weights(tn, hn)
        acc = lsum = mx = None
        ss = []

        def qk(c):
            nonlocal mx
            s = -_dot(_upk(k_scr[gn, c * CK // 2:(c + 1) * CK // 2, :]), qm)
            dst[0, c * CK:(c + 1) * CK, :] = s
            ss.append(s)
            cm = _tree(s, jnp.minimum)
            mx = cm if mx is None else jnp.minimum(mx, cm)

        for c in range(SKEW_SLOW):
            qk(c)
        m = m_cur
        for c in range(NC):
            if c >= 1:
                gc, gr = divmod(c * 16 + GATE_SLOW, 16)
                m = _after(m, jnp.concatenate([ss[gc][gr * 8:(gr + 1) * 8, 384:512]] * 4, axis=1))
            p = probs(c, m, src, z, slice(0, TQ))
            ls = _tree(p, jnp.add)
            lsum = ls if lsum is None else lsum + ls
            pv = _dot(v_rows(h, c, False), p.astype(bf16))
            acc = pv if acc is None else acc + pv
            if c + SKEW_SLOW < NC:
                qk(c + SKEW_SLOW)
        l = jnp.sum(lsum, axis=0, keepdims=True)
        oT_scr[pl.ds(pl.multiple_of(h * DH, DH), DH), :] = acc * (1.0 / l)
        return _allred8(mx, jnp.minimum)

    def ffn_units(j):
        rows = half_rows(j * FR, FR)
        out_rows = pl.ds(pl.multiple_of(j * FR, FR), FR)
        st = {}

        def gate_up(fc, w_ref, kh):
            ks, cs = slice(kh * 256, (kh + 1) * 256), slice(fc * 128, (fc + 1) * 128)
            r = _dot(_upk(hn_scr[rows, ks]), w_ref[ks, cs])
            if kh == 0:
                st["part"] = r
            elif w_ref is wg_ref:
                st["g"] = r + st.pop("part")
            else:
                g, u = st.pop("g"), r + st.pop("part")
                a = g * u * (0.5 * jnp.tanh(0.5 * g) + 0.5)
                a_scr[:, cs] = _pk(a.astype(bf16))

        def down(oc, kh):
            ks, cs = slice(kh * 256, (kh + 1) * 256), slice(oc * 128, (oc + 1) * 128)
            y = _dot(_upk(a_scr[:, ks]), wd_ref[ks, cs])
            if kh > 0:
                y = y + st.pop("y")
            if kh < F // 256 - 1:
                st["y"] = y
            else:
                o_ref[out_rows, cs] = (h1_scr[out_rows, cs] + y).astype(o_ref.dtype)

        units = [functools.partial(gate_up, fc, w_ref, kh)
                 for fc in range(F // 128) for w_ref in (wg_ref, wu_ref) for kh in range(2)]
        units += [functools.partial(down, oc, kh) for oc in range(4) for kh in range(F // 256)]
        return units

    def heads_loop(head_fn, unroll, with_ffn=False):
        def body(j, m):
            z = flag_ref[0]
            slots = {}
            if with_ffn:
                units = ffn_units(j)
                for n, fn in enumerate(units):
                    step = int(2 + n / len(units) * (unroll * NC - 6))
                    slots.setdefault(2 * step + n % 2, []).append(fn)
            for u in range(unroll):
                src, dst = (s_a, s_b) if u % 2 == 0 else (s_b, s_a)
                args = (j * unroll + u, m, src, dst, z)
                if with_ffn:
                    def hook(pos, u=u):
                        for fn in slots.get(u * NC * 2 + pos, []):
                            fn()
                    m = head_fn(*args, hook)
                else:
                    m = head_fn(*args)
            return m
        m_scr[...] = lax.fori_loop(0, H // unroll, body, m_scr[...])

    fast = flag_ref[1] == 1

    @pl.when(i == 1)
    def _():
        for cp in w_copies()[1:]:
            cp.wait()

    @pl.when(jnp.logical_and(fast, i == 0))
    def _():
        heads_loop(fast_head, UNR_FAST)

    @pl.when(jnp.logical_and(fast, jnp.logical_and(i > 0, i < NQ)))
    def _():
        heads_loop(fast_head, UNR_FAST, with_ffn=True)

    @pl.when(jnp.logical_or(i == NQ, jnp.logical_and(i > 0, jnp.logical_not(fast))))
    def _():
        def ffn_body(j, carry):
            for fn in ffn_units(j):
                fn()
            return carry
        lax.fori_loop(0, TQ // FR, ffn_body, 0)

    @pl.when(jnp.logical_and(jnp.logical_not(fast), i < NQ))
    def _():
        heads_loop(slow_head, UNR_SLOW)

    @pl.when(i == 0)
    def _():
        w_copies()[0].wait()

    @pl.when(i < NQ)
    def _():
        for b in range(TQ // FR):
            r0 = pl.multiple_of(i * TQ + b * FR, FR)
            o = oT_scr[:, b * FR:(b + 1) * FR].T.astype(bf16)
            h1 = x_ref[pl.ds(r0, FR), :].astype(f32) + _dot(o, wo_ref[...])
            h1_scr[b * FR:(b + 1) * FR, :] = h1
            hn_scr[b * FR // 2:(b + 1) * FR // 2, :] = _pk(_ln(h1).astype(bf16))


@jax.jit
def pallas_sequential_preLN__softmax_full_mha__swiglu_ffn__prompt_kernel(
    A_x: jax.Array,
    A_wqkv: jax.Array,
    A_wo: jax.Array,
    B_x: jax.Array,
    B_w_gate: jax.Array,
    B_w_up: jax.Array,
    B_w_down: jax.Array,
):
    del B_x
    out = pl.pallas_call(
        _kernel,
        grid=(NQ + 1,),
        in_specs=[pl.BlockSpec(memory_space=pl.ANY)] * 6,
        out_specs=pl.BlockSpec((TQ, D), lambda i: (jnp.maximum(i - 1, 0), 0)),
        out_shape=jax.ShapeDtypeStruct((S, D), bf16),
        scratch_shapes=[
            pltpu.VMEM((S, D), bf16),
            pltpu.VMEM((D, 3 * D), bf16),
            pltpu.VMEM((D, D), bf16),
            pltpu.VMEM((D, F), bf16),
            pltpu.VMEM((D, F), bf16),
            pltpu.VMEM((F, D), bf16),
            pltpu.SemaphoreType.DMA((NQ + 7,)),
            pltpu.VMEM((3 * D // 2, D), u32),
            pltpu.VMEM((S // 2, D), u32),
            pltpu.VMEM((S // 2, D), u32),
            pltpu.VMEM((2, 4, TQ, 128), f32),
            pltpu.VMEM((NQ, D, TQ), f32),
            pltpu.VMEM((H, 8, 128), f32),
            pltpu.VMEM((H, S // 4, 128), u32),
            pltpu.VMEM((NQ, H, QROWS // 4, TQ), u32),
            pltpu.VMEM((NQ, H, 8, TQ), i32),
            pltpu.VMEM((NQ, H, 16, TQ), u32),
            pltpu.VMEM((4, S // 2, 128), u32),
            pltpu.VMEM((S // QB, D // 2, QB), u32),
            pltpu.VMEM((1, S, TQ), f32),
            pltpu.VMEM((1, S, TQ), f32),
            pltpu.VMEM((8, TQ), f32),
            pltpu.VMEM((D, TQ), f32),
            pltpu.VMEM((TQ, D), f32),
            pltpu.VMEM((TQ // 2, D), u32),
            pltpu.VMEM((FR // 2, F), u32),
            pltpu.SMEM((2,), i32),
        ],
        compiler_params=pltpu.CompilerParams(
            dimension_semantics=("arbitrary",),
            vmem_limit_bytes=110 * 1024 * 1024,
        ),
    )(A_x.reshape(S, D), A_wqkv, A_wo, B_w_gate, B_w_up, B_w_down)
    return out.reshape(1, S, D)
```

```python
import functools
import math

import jax
import jax.numpy as jnp
from jax import lax
from jax.experimental import pallas as pl
from jax.experimental.pallas import tpu as pltpu

S, D, H, DH, F = 2048, 512, 32, 16, 1792
TQ = 512
HW = TQ // 2
CK = 128
NC = S // CK
NQ = S // TQ
QB = 128
FR = 128
UNR_FAST = H * FR // TQ
UNR_SLOW = 2
SKEW_SOLO, GATE_SOLO = 3, -8
SKEW_FUSE, GATE_FUSE = 2, -56
SKEW_SLOW, GATE_SLOW = 2, -12
LEVELS = (2, 4)
NT = 1 + 2 * len(LEVELS)
QROWS = -(-NT * DH // 32) * 32
EPS = 1e-5
QSCALE = (DH ** -0.5) * math.log2(math.e)
UNIT_MAX = 2.0 ** -9
RMAGIC = 12582912.0

bf16 = jnp.bfloat16
f32 = jnp.float32
u32 = jnp.uint32
i32 = jnp.int32
i8 = jnp.int8


def _pk(x):
    return pltpu.bitcast(x, u32)


def _upk(x):
    return pltpu.bitcast(x, bf16)


def _tree(x, op):
    parts = [x[8 * j:8 * (j + 1)] for j in range(x.shape[0] // 8)]
    while len(parts) > 1:
        parts = [op(parts[2 * j], parts[2 * j + 1]) for j in range(len(parts) // 2)]
    return parts[0]


def _allred8(m, op):
    for sh in (4, 2, 1):
        m = op(m, pltpu.roll(m, sh, 0))
    return m


def _after(x, dep):
    return jnp.minimum(x, jnp.maximum(x, dep))


def _after_rows(x, dep):
    dep = jnp.concatenate([dep] * (x.shape[1] // 128), axis=1)
    head = _after(pltpu.bitcast(x[0:8], i32), dep)
    return jnp.concatenate([pltpu.bitcast(head, u32), x[8:]], axis=0)


def _ln(x):
    mu = jnp.mean(x, axis=-1, keepdims=True)
    xc = x - mu
    var = jnp.mean(xc * xc, axis=-1, keepdims=True)
    return xc * lax.rsqrt(var + EPS)


def _dot(a, b):
    return jnp.dot(a, b, preferred_element_type=f32)


def _dot_nt(a, b):
    return lax.dot_general(a, b, (((1,), (1,)), ((), ())), preferred_element_type=f32)


def _rbits(v, a):
    return pltpu.bitcast(v + RMAGIC * 2.0 ** -a, i32)


def _limbs(x):
    prev, a_prev = _rbits(x, 0), 0
    main, fine, coarse = prev, [], []
    for a in LEVELS:
        r = _rbits(x, a)
        fine.append(r - (prev << (a - a_prev)))
        coarse.append(_rbits(x, -a))
        prev, a_prev = r, a
    return main, fine, coarse


def _kernel(x_hbm, wqkv_hbm, wo_hbm, wg_hbm, wu_hbm, wd_hbm, o_ref,
            x_ref, wqkv_ref, wo_ref, wg_ref, wu_ref, wd_ref, sems,
            wT_scr, xp_scr, xn_scr, xf_scr, kT_scr, kmax_scr, k8_scr, q8_scr, b_scr, vT_scr,
            k_scr, qT_scr, s_a, s_b, m_scr, oT_scr, h1_scr, hn_scr, a_scr, flag_ref):
    i = pl.program_id(0)

    def x_copy(t):
        rows = pl.ds(t * TQ, TQ)
        return pltpu.make_async_copy(x_hbm.at[rows, :], x_ref.at[rows, :], sems.at[t])

    def wqkv_copy(j):
        cols = pl.ds(j * D, D)
        return pltpu.make_async_copy(wqkv_hbm.at[:, cols], wqkv_ref.at[:, cols], sems.at[NQ + j])

    def w_copy(j):
        src, dst = ((wo_hbm, wo_ref), (wg_hbm, wg_ref), (wu_hbm, wu_ref), (wd_hbm, wd_ref))[j]
        return pltpu.make_async_copy(src, dst, sems.at[NQ + 3 + j])

    def half_rows(start, n):
        return pl.ds(pl.multiple_of(start // 2, n // 2), n // 2)

    def transposed_weight(j):
        return _pk(wqkv_ref[:, j * D:(j + 1) * D].astype(f32).T.astype(bf16))


    def fast_weights(tile, h):
        w = jnp.concatenate([q8_scr[tile, h], jnp.zeros(((128 - QROWS) // 4, TQ), u32)], axis=0)
        return pltpu.bitcast(w, i8)

    def fast_scores(kc, qm, bv):
        v = jnp.dot(pltpu.bitcast(kc, i8), qm, preferred_element_type=i32)
        n = v.shape[1]
        return pltpu.bitcast((bv[None] - v.reshape(CK // 8, 8, n)).reshape(CK, n), f32)

    def slow_weights(tile, h):
        g8 = pl.multiple_of(lax.shift_right_logical(h, 3) * 64, 64)
        nb = TQ // QB
        qg = jnp.concatenate([qT_scr[tile * nb + b, pl.ds(g8, 64), :] for b in range(nb)], axis=1)
        row = lax.shift_right_logical(lax.broadcasted_iota(i32, (64, TQ), 0), 3)
        return _upk(jnp.where(row == (h & 7), qg, jnp.zeros_like(qg)))

    @pl.when(i == 0)
    def _():
        wqkv_copy(1).start()
        x_copy(0).start()
        flag_ref[0] = 0
        kmax_scr[...] = jnp.zeros_like(kmax_scr)
        ones_row = jnp.where(lax.broadcasted_iota(i32, (8, TQ), 0) == 0,
                             jnp.uint32(0x3F80), jnp.uint32(0))
        for t in range(NQ):
            for h in range(H):
                vT_scr[t, h, 8:16, :] = ones_row
        wqkv_copy(1).wait()
        x_copy(0).wait()
        for t in range(1, NQ):
            x_copy(t).start()
        wqkv_copy(0).start()
        wqkv_copy(2).start()
        wT_scr[0:D // 2, :] = transposed_weight(1)

        for t in range(NQ):
            if t == 1:
                x_copy(1).wait()
                x_copy(2).wait()
            if t == 3:
                x_copy(3).wait()
                wqkv_copy(0).wait()
                wqkv_copy(2).wait()
                for j in range(4):
                    w_copy(j).start()
            for b in range(TQ // QB):
                r0 = t * TQ + b * QB
                xn = _ln(x_ref[r0:r0 + QB, :].astype(f32))
                for g in range(4):
                    xf_scr[t % 2, g, pl.ds(b, QB, stride=4), :] = xn[:, g * 128:(g + 1) * 128]
                xn = xn.astype(bf16)
                xn_scr[r0 // 2:(r0 + QB) // 2, :] = _pk(xn)
                kt = _dot_nt(_upk(wT_scr[0:D // 2, :]), xn)
                kT_scr[t, :, b * QB:(b + 1) * QB] = kt
                ka = jnp.abs(kt).reshape(H, 2, 8, QB)
                kmax_scr[...] = jnp.maximum(kmax_scr[...], jnp.maximum(ka[:, 0], ka[:, 1]))
            for b in range(TQ // QB):
                r0 = t * TQ + b * QB
                xp = jnp.concatenate([xf_scr[t % 2, g, b * QB:(b + 1) * QB, :] for g in range(4)], axis=1)
                xp_scr[r0 // 2:(r0 + QB) // 2, :] = _pk(xp.astype(bf16))
        wT_scr[D // 2:D, :] = transposed_weight(0)
        wT_scr[D:3 * D // 2, :] = transposed_weight(2)

        km = jnp.max(kmax_scr[...], axis=2, keepdims=True)
        km = jnp.maximum(jnp.max(km, axis=1, keepdims=True), 1e-30)
        kmax_scr[...] = jnp.broadcast_to(km, (H, 8, 128))

        def quant_k(t, h):
            kinv = jnp.concatenate([127.0 / kmax_scr[h]] * 4, axis=1)
            y = kT_scr[t, h * DH:(h + 1) * DH, :]
            y = (y.reshape(2, 8, TQ) * kinv[None]).reshape(DH, TQ)
            main, fine, coarse = _limbs(y)
            words = [((v[:, 0:128] & 0xFF) | ((v[:, 128:256] & 0xFF) << 8)
                      | ((v[:, 256:384] & 0xFF) << 16) | (v[:, 384:512] << 24))
                     for v in [main] + coarse + fine]
            words.append(jnp.zeros((128 - NT * DH, 128), i32))
            wt = jnp.concatenate(words, axis=0).T
            k8_scr[h, pl.ds(pl.multiple_of(t * 128, 128), 128), :] = pltpu.bitcast(wt, u32)
            return wt[120:128]

        def body_b(t, umax):
            for b in range(TQ // QB):
                rows = half_rows(t * TQ + b * QB, QB)
                qt = _dot_nt(_upk(wT_scr[D // 2:D, :]), _upk(xn_scr[rows, :]))
                dep = functools.reduce(jnp.bitwise_or, [quant_k(t, h) for h in range(b * 8, b * 8 + 8)])
                for h in range(H):
                    q = qt[h * DH:(h + 1) * DH]
                    kmx = kmax_scr[h]
                    qa = jnp.abs(q)
                    qmx = _allred8(jnp.maximum(qa[0:8], qa[8:16]), jnp.maximum)
                    uraw = jnp.maximum(qmx * kmx * (QSCALE / (127.0 * 127.0)), 2.0 ** -60)
                    umax = jnp.maximum(umax, uraw)
                    ub = (pltpu.bitcast(uraw, i32) + 0x7FFFFF) & 0x7F800000
                    b_scr[t, h, :, b * QB:(b + 1) * QB] = ub + ((23 << 23) + (1 << 22))
                    sc = kmx * pltpu.bitcast((254 << 23) - ub, f32) * (QSCALE / 127.0)
                    main, fine, coarse = _limbs((q.reshape(2, 8, QB) * sc[None]).reshape(DH, QB))
                    limbs = [main] + fine + coarse + [jnp.zeros((QROWS - NT * DH, QB), i32)]
                    q8_scr[t, h, :, b * QB:(b + 1) * QB] = _pk(jnp.concatenate(limbs, axis=0).astype(i8))
                xp = _upk(_after_rows(xp_scr[rows, :], dep))
                vb = _pk(_dot_nt(_upk(wT_scr[D:3 * D // 2, :]), xp).astype(bf16))
                for h in range(H):
                    vT_scr[t, h, 0:8, b * QB:(b + 1) * QB] = vb[h * 8:(h + 1) * 8]
            return umax
        umax = lax.fori_loop(0, NQ, body_b, jnp.zeros((8, QB), f32))
        flag_ref[1] = jnp.where(jnp.max(umax) <= UNIT_MAX, 1, 0).astype(i32)

        @pl.when(flag_ref[1] == 1)
        def _():
            qm, bv, mx = fast_weights(0, 0), b_scr[0, 0], None
            for c in range(NC):
                s = fast_scores(k8_scr[0, c * CK // 4:(c + 1) * CK // 4, :], qm, bv)
                s_a[0, c * CK:(c + 1) * CK, :] = s
                cm = _tree(s, jnp.minimum)
                mx = cm if mx is None else jnp.minimum(mx, cm)
            m_scr[...] = _allred8(mx, jnp.minimum)

        @pl.when(flag_ref[1] == 0)
        def _():
            def body_s(t, carry):
                rows = half_rows(t * QB, QB)
                kk = _dot(_upk(xp_scr[rows, :]), wqkv_ref[:, D:2 * D]).astype(bf16)
                for g in range(4):
                    k_scr[g, rows, :] = _pk(kk[:, g * 128:(g + 1) * 128])
                qq = _dot_nt(_upk(wT_scr[D // 2:D, :]), _upk(xn_scr[rows, :]))
                qT_scr[t] = _pk((qq * QSCALE).astype(bf16))
                return carry
            lax.fori_loop(0, S // QB, body_s, 0)
            qm = slow_weights(0, 0)

            def body_p(c, mx):
                s = -_dot(_upk(k_scr[0, half_rows(c * CK, CK), :]), qm)
                s_a[0, pl.ds(pl.multiple_of(c * CK, CK), CK), :] = s
                return jnp.minimum(mx, _tree(s, jnp.minimum))
            mx = lax.fori_loop(0, NC, body_p, jnp.full((8, TQ), jnp.inf, f32))
            m_scr[...] = _allred8(mx, jnp.minimum)

    def next_head(h):
        hn = (h + 1) & (H - 1)
        tn = jnp.minimum(i + lax.shift_right_logical(h + 1, 5), NQ - 1)
        return hn, tn

    def probs(c, m, src, z, cols):
        n = cols.stop - cols.start
        sv = src[z, c * CK:(c + 1) * CK, cols].reshape(CK // 8, 8, n)
        return jnp.exp2(m[None] - sv).reshape(CK, n)

    def v_rows(h, c, with_ones):
        t, cc = divmod(c * CK, TQ)
        return _upk(vT_scr[t, h, 0:(16 if with_ones else 8), cc:cc + CK])

    def fast_head(h, m_cur, src, dst, z, hook=None):
        solo = hook is None
        skew, gate = (SKEW_SOLO, GATE_SOLO) if solo else (SKEW_FUSE, GATE_FUSE)
        hn, tn = next_head(h)
        qm, bv = fast_weights(tn, hn), b_scr[tn, hn]
        cols = [slice(s * HW, (s + 1) * HW) for s in range(2)]
        st = [dict(mx=None, acc=None, ss=[], m=m_cur[:, cols[s]]) for s in range(2)]

        def qk(s, c):
            kc = k8_scr[hn, c * CK // 4:(c + 1) * CK // 4, :]
            if solo and s == 1 and c >= 1:
                kc = _after_rows(kc, pltpu.bitcast(st[0]["ss"][c - 1][0:8, 0:128], i32))
            v = fast_scores(kc, qm[:, cols[s]], bv[:, cols[s]])
            dst[0, c * CK:(c + 1) * CK, cols[s]] = v
            d = st[s]
            d["ss"].append(v)
            cm = _tree(v, jnp.minimum)
            d["mx"] = cm if d["mx"] is None else jnp.minimum(d["mx"], cm)

        for c in range(skew):
            for s in range(2):
                qk(s, c)
        for c in range(NC):
            for s in range(2):
                d = st[s]
                gc, gr = divmod(c * 16 + gate, 16)
                if gc >= 0:
                    dep = d["ss"][gc][gr * 8:(gr + 1) * 8, 128:256]
                    d["m"] = _after(d["m"], jnp.concatenate([dep] * 2, axis=1))
                p = probs(c, d["m"], src, z, cols[s])
                pv = _dot(v_rows(h, c, solo), p.astype(bf16))
                pv = pv[0:24] if solo else jnp.concatenate([pv, _tree(p, jnp.add)], axis=0)
                d["acc"] = pv if d["acc"] is None else d["acc"] + pv
            for s in range(2):
                if not solo:
                    hook(2 * c + s)
                if c + skew < NC:
                    qk(s, c + skew)
        acc = jnp.concatenate([st[0]["acc"], st[1]["acc"]], axis=1)
        l = acc[16:17] if solo else jnp.sum(acc[16:24], axis=0, keepdims=True)
        oT_scr[pl.ds(pl.multiple_of(h * DH, DH), DH), :] = acc[0:16] * (1.0 / l)
        return _allred8(jnp.concatenate([st[0]["mx"], st[1]["mx"]], axis=1), jnp.minimum)

    def slow_head(h, m_cur, src, dst, z):
        hn, tn = next_head(h)
        gn = lax.shift_right_logical(hn, 3)
        qm = slow_weights(tn, hn)
        acc = lsum = mx = None
        ss = []

        def qk(c):
            nonlocal mx
            s = -_dot(_upk(k_scr[gn, c * CK // 2:(c + 1) * CK // 2, :]), qm)
            dst[0, c * CK:(c + 1) * CK, :] = s
            ss.append(s)
            cm = _tree(s, jnp.minimum)
            mx = cm if mx is None else jnp.minimum(mx, cm)

        for c in range(SKEW_SLOW):
            qk(c)
        m = m_cur
        for c in range(NC):
            if c >= 1:
                gc, gr = divmod(c * 16 + GATE_SLOW, 16)
                m = _after(m, jnp.concatenate([ss[gc][gr * 8:(gr + 1) * 8, 384:512]] * 4, axis=1))
            p = probs(c, m, src, z, slice(0, TQ))
            ls = _tree(p, jnp.add)
            lsum = ls if lsum is None else lsum + ls
            pv = _dot(v_rows(h, c, False), p.astype(bf16))
            acc = pv if acc is None else acc + pv
            if c + SKEW_SLOW < NC:
                qk(c + SKEW_SLOW)
        l = jnp.sum(lsum, axis=0, keepdims=True)
        oT_scr[pl.ds(pl.multiple_of(h * DH, DH), DH), :] = acc * (1.0 / l)
        return _allred8(mx, jnp.minimum)

    def ffn_units(j):
        rows = half_rows(j * FR, FR)
        out_rows = pl.ds(pl.multiple_of(j * FR, FR), FR)
        st = {}

        def gate_up(fc, w_ref, kh):
            ks, cs = slice(kh * 256, (kh + 1) * 256), slice(fc * 128, (fc + 1) * 128)
            r = _dot(_upk(hn_scr[rows, ks]), w_ref[ks, cs])
            if kh == 0:
                st["part"] = r
            elif w_ref is wg_ref:
                st["g"] = r + st.pop("part")
            else:
                g, u = st.pop("g"), r + st.pop("part")
                a = g * u * (0.5 * jnp.tanh(0.5 * g) + 0.5)
                a_scr[:, cs] = _pk(a.astype(bf16))

        def down(oc, kh):
            ks, cs = slice(kh * 256, (kh + 1) * 256), slice(oc * 128, (oc + 1) * 128)
            y = _dot(_upk(a_scr[:, ks]), wd_ref[ks, cs])
            if kh > 0:
                y = y + st.pop("y")
            if kh < F // 256 - 1:
                st["y"] = y
            else:
                o_ref[out_rows, cs] = (h1_scr[out_rows, cs] + y).astype(o_ref.dtype)

        units = [functools.partial(gate_up, fc, w_ref, kh)
                 for fc in range(F // 128) for w_ref in (wg_ref, wu_ref) for kh in range(2)]
        units += [functools.partial(down, oc, kh) for oc in range(4) for kh in range(F // 256)]
        return units

    def heads_loop(head_fn, unroll, with_ffn=False):
        def body(j, m):
            z = flag_ref[0]
            slots = {}
            if with_ffn:
                units = ffn_units(j)
                for n, fn in enumerate(units):
                    step = int(2 + n / len(units) * (unroll * NC - 4))
                    slots.setdefault(2 * step + n % 2, []).append(fn)
            for u in range(unroll):
                src, dst = (s_a, s_b) if u % 2 == 0 else (s_b, s_a)
                args = (j * unroll + u, m, src, dst, z)
                if with_ffn:
                    def hook(pos, u=u):
                        for fn in slots.get(u * NC * 2 + pos, []):
                            fn()
                    m = head_fn(*args, hook)
                else:
                    m = head_fn(*args)
            return m
        m_scr[...] = lax.fori_loop(0, H // unroll, body, m_scr[...])

    fast = flag_ref[1] == 1

    @pl.when(i == 1)
    def _():
        for j in range(1, 4):
            w_copy(j).wait()

    @pl.when(jnp.logical_and(fast, i == 0))
    def _():
        heads_loop(fast_head, UNR_FAST)

    @pl.when(jnp.logical_and(fast, jnp.logical_and(i > 0, i < NQ)))
    def _():
        heads_loop(fast_head, UNR_FAST, with_ffn=True)

    @pl.when(jnp.logical_or(i == NQ, jnp.logical_and(i > 0, jnp.logical_not(fast))))
    def _():
        def ffn_body(j, carry):
            for fn in ffn_units(j):
                fn()
            return carry
        lax.fori_loop(0, TQ // FR, ffn_body, 0)

    @pl.when(jnp.logical_and(jnp.logical_not(fast), i < NQ))
    def _():
        heads_loop(slow_head, UNR_SLOW)

    @pl.when(i == 0)
    def _():
        w_copy(0).wait()

    @pl.when(i < NQ)
    def _():
        for b in range(TQ // FR):
            r0 = pl.multiple_of(i * TQ + b * FR, FR)
            o = oT_scr[:, b * FR:(b + 1) * FR].T.astype(bf16)
            h1 = x_ref[pl.ds(r0, FR), :].astype(f32) + _dot(o, wo_ref[...])
            h1_scr[b * FR:(b + 1) * FR, :] = h1
            hn_scr[b * FR // 2:(b + 1) * FR // 2, :] = _pk(_ln(h1).astype(bf16))


@jax.jit
def pallas_sequential_preLN__softmax_full_mha__swiglu_ffn__prompt_kernel(
    A_x: jax.Array,
    A_wqkv: jax.Array,
    A_wo: jax.Array,
    B_x: jax.Array,
    B_w_gate: jax.Array,
    B_w_up: jax.Array,
    B_w_down: jax.Array,
):
    del B_x
    out = pl.pallas_call(
        _kernel,
        grid=(NQ + 1,),
        in_specs=[pl.BlockSpec(memory_space=pl.ANY)] * 6,
        out_specs=pl.BlockSpec((TQ, D), lambda i: (jnp.maximum(i - 1, 0), 0)),
        out_shape=jax.ShapeDtypeStruct((S, D), bf16),
        scratch_shapes=[
            pltpu.VMEM((S, D), bf16),
            pltpu.VMEM((D, 3 * D), bf16),
            pltpu.VMEM((D, D), bf16),
            pltpu.VMEM((D, F), bf16),
            pltpu.VMEM((D, F), bf16),
            pltpu.VMEM((F, D), bf16),
            pltpu.SemaphoreType.DMA((NQ + 7,)),
            pltpu.VMEM((3 * D // 2, D), u32),
            pltpu.VMEM((S // 2, D), u32),
            pltpu.VMEM((S // 2, D), u32),
            pltpu.VMEM((2, 4, TQ, 128), f32),
            pltpu.VMEM((NQ, D, TQ), f32),
            pltpu.VMEM((H, 8, 128), f32),
            pltpu.VMEM((H, S // 4, 128), u32),
            pltpu.VMEM((NQ, H, QROWS // 4, TQ), u32),
            pltpu.VMEM((NQ, H, 8, TQ), i32),
            pltpu.VMEM((NQ, H, 16, TQ), u32),
            pltpu.VMEM((4, S // 2, 128), u32),
            pltpu.VMEM((S // QB, D // 2, QB), u32),
            pltpu.VMEM((1, S, TQ), f32),
            pltpu.VMEM((1, S, TQ), f32),
            pltpu.VMEM((8, TQ), f32),
            pltpu.VMEM((D, TQ), f32),
            pltpu.VMEM((TQ, D), f32),
            pltpu.VMEM((TQ // 2, D), u32),
            pltpu.VMEM((FR // 2, F), u32),
            pltpu.SMEM((2,), i32),
        ],
        compiler_params=pltpu.CompilerParams(
            dimension_semantics=("arbitrary",),
            vmem_limit_bytes=110 * 1024 * 1024,
        ),
    )(A_x.reshape(S, D), A_wqkv, A_wo, B_w_gate, B_w_up, B_w_down)
    return out.reshape(1, S, D)
```

```python
import functools
import math

import jax
import jax.numpy as jnp
from jax import lax
from jax.experimental import pallas as pl
from jax.experimental.pallas import tpu as pltpu

S, D, H, DH, F = 2048, 512, 32, 16, 1792
TQ = 512
HW = TQ // 2
CK = 128
NC = S // CK
NQ = S // TQ
QB = 128
FR = 128
UNR_FAST = H * FR // TQ
UNR_SLOW = 2
SKEW_SOLO, GATE_SOLO = 3, -8
SKEW_FUSE, GATE_FUSE = 2, -56
SKEW_SLOW, GATE_SLOW = 2, -12
LEVELS = (2, 4)
NT = 1 + 2 * len(LEVELS)
QROWS = -(-NT * DH // 32) * 32
EPS = 1e-5
QSCALE = (DH ** -0.5) * math.log2(math.e)
UNIT_MAX = 2.0 ** -9
RMAGIC = 12582912.0

bf16 = jnp.bfloat16
f32 = jnp.float32
u32 = jnp.uint32
i32 = jnp.int32
i8 = jnp.int8


def _pk(x):
    return pltpu.bitcast(x, u32)


def _upk(x):
    return pltpu.bitcast(x, bf16)


def _tree(x, op):
    parts = [x[8 * j:8 * (j + 1)] for j in range(x.shape[0] // 8)]
    while len(parts) > 1:
        parts = [op(parts[2 * j], parts[2 * j + 1]) for j in range(len(parts) // 2)]
    return parts[0]


def _allred8(m, op):
    for sh in (4, 2, 1):
        m = op(m, pltpu.roll(m, sh, 0))
    return m


def _after(x, dep):
    return jnp.minimum(x, jnp.maximum(x, dep))


def _after_rows(x, dep):
    dep = jnp.concatenate([dep] * (x.shape[1] // 128), axis=1)
    head = _after(pltpu.bitcast(x[0:8], i32), dep)
    return jnp.concatenate([pltpu.bitcast(head, u32), x[8:]], axis=0)


def _ln(x):
    mu = jnp.mean(x, axis=-1, keepdims=True)
    xc = x - mu
    var = jnp.mean(xc * xc, axis=-1, keepdims=True)
    return xc * lax.rsqrt(var + EPS)


def _dot(a, b):
    return jnp.dot(a, b, preferred_element_type=f32)


def _dot_nt(a, b):
    return lax.dot_general(a, b, (((1,), (1,)), ((), ())), preferred_element_type=f32)


def _rbits(v, a):
    return pltpu.bitcast(v + RMAGIC * 2.0 ** -a, i32)


def _limbs(x):
    prev, a_prev = _rbits(x, 0), 0
    main, fine, coarse = prev, [], []
    for a in LEVELS:
        r = _rbits(x, a)
        fine.append(r - (prev << (a - a_prev)))
        coarse.append(_rbits(x, -a))
        prev, a_prev = r, a
    return main, fine, coarse


def _kernel(x_hbm, wqkv_hbm, wo_hbm, wg_hbm, wu_hbm, wd_hbm, o_ref,
            x_ref, wqkv_ref, wo_ref, wg_ref, wu_ref, wd_ref, sems,
            wT_scr, xp_scr, xn_scr, xf_scr, kT_scr, kmax_scr, k8_scr, q8_scr, b_scr, vT_scr,
            k_scr, qT_scr, s_a, s_b, m_scr, oT_scr, h1_scr, hn_scr, a_scr, flag_ref):
    i = pl.program_id(0)

    def x_copy(t):
        rows = pl.ds(t * TQ, TQ)
        return pltpu.make_async_copy(x_hbm.at[rows, :], x_ref.at[rows, :], sems.at[t])

    def wqkv_copy(j):
        cols = pl.ds(j * D, D)
        return pltpu.make_async_copy(wqkv_hbm.at[:, cols], wqkv_ref.at[:, cols], sems.at[NQ + j])

    def w_copy(j):
        src, dst = ((wo_hbm, wo_ref), (wg_hbm, wg_ref), (wu_hbm, wu_ref), (wd_hbm, wd_ref))[j]
        return pltpu.make_async_copy(src, dst, sems.at[NQ + 3 + j])

    def half_rows(start, n):
        return pl.ds(pl.multiple_of(start // 2, n // 2), n // 2)

    def transposed_weight(j):
        return _pk(wqkv_ref[:, j * D:(j + 1) * D].astype(f32).T.astype(bf16))


    def fast_weights(tile, h):
        w = jnp.concatenate([q8_scr[tile, h], jnp.zeros(((128 - QROWS) // 4, TQ), u32)], axis=0)
        return pltpu.bitcast(w, i8)

    def fast_scores(kc, qm, bv):
        v = jnp.dot(pltpu.bitcast(kc, i8), qm, preferred_element_type=i32)
        n = v.shape[1]
        return pltpu.bitcast((bv[None] - v.reshape(CK // 8, 8, n)).reshape(CK, n), f32)

    def slow_weights(tile, h):
        g8 = pl.multiple_of(lax.shift_right_logical(h, 3) * 64, 64)
        nb = TQ // QB
        qg = jnp.concatenate([qT_scr[tile * nb + b, pl.ds(g8, 64), :] for b in range(nb)], axis=1)
        row = lax.shift_right_logical(lax.broadcasted_iota(i32, (64, TQ), 0), 3)
        return _upk(jnp.where(row == (h & 7), qg, jnp.zeros_like(qg)))

    @pl.when(i == 0)
    def _():
        wqkv_copy(1).start()
        for t in range(3):
            x_copy(t).start()
        flag_ref[0] = 0
        kmax_scr[...] = jnp.zeros_like(kmax_scr)
        ones_row = jnp.where(lax.broadcasted_iota(i32, (8, TQ), 0) == 0,
                             jnp.uint32(0x3F80), jnp.uint32(0))
        for t in range(NQ):
            for h in range(H):
                vT_scr[t, h, 8:16, :] = ones_row
        wqkv_copy(1).wait()
        x_copy(0).wait()
        x_copy(3).start()
        wqkv_copy(0).start()
        wqkv_copy(2).start()
        wT_scr[0:D // 2, :] = transposed_weight(1)

        nb = TQ // QB

        def ln_block(sb):
            t, b = divmod(sb, nb)
            r0 = sb * QB
            xn = _ln(x_ref[r0:r0 + QB, :].astype(f32))
            for g in range(4):
                xf_scr[t % 2, g, pl.ds(b, QB, stride=4), :] = xn[:, g * 128:(g + 1) * 128]
            xn = xn.astype(bf16)
            xn_scr[r0 // 2:(r0 + QB) // 2, :] = _pk(xn)
            if b == nb - 1:
                for bb in range(nb):
                    rr = t * TQ + bb * QB
                    xp = jnp.concatenate([xf_scr[t % 2, g, bb * QB:(bb + 1) * QB, :] for g in range(4)], axis=1)
                    xp_scr[rr // 2:(rr + QB) // 2, :] = _pk(xp.astype(bf16))
            return xn

        def k_block(sb, xn):
            t, b = divmod(sb, nb)
            kt = _dot_nt(_upk(wT_scr[0:D // 2, :]), xn)
            kT_scr[t, :, b * QB:(b + 1) * QB] = kt
            ka = jnp.abs(kt).reshape(H, 2, 8, QB)
            kmax_scr[...] = jnp.maximum(kmax_scr[...], jnp.maximum(ka[:, 0], ka[:, 1]))

        held = None
        for sb in range(S // QB):
            if sb == nb:
                x_copy(1).wait()
                x_copy(2).wait()
            if sb == 3 * nb:
                x_copy(3).wait()
                wqkv_copy(0).wait()
                wqkv_copy(2).wait()
                for j in range(4):
                    w_copy(j).start()
            if held is not None:
                k_block(*held)
                held = None
            xn = ln_block(sb)
            if sb + 1 in (nb, 3 * nb):
                held = (sb, xn)
            else:
                k_block(sb, xn)
        wT_scr[D // 2:D, :] = transposed_weight(0)
        wT_scr[D:3 * D // 2, :] = transposed_weight(2)

        km = jnp.max(kmax_scr[...], axis=2, keepdims=True)
        km = jnp.maximum(jnp.max(km, axis=1, keepdims=True), 1e-30)
        kmax_scr[...] = jnp.broadcast_to(km, (H, 8, 128))

        def quant_k(t, h):
            kinv = jnp.concatenate([127.0 / kmax_scr[h]] * 4, axis=1)
            y = kT_scr[t, h * DH:(h + 1) * DH, :]
            y = (y.reshape(2, 8, TQ) * kinv[None]).reshape(DH, TQ)
            main, fine, coarse = _limbs(y)
            words = [((v[:, 0:128] & 0xFF) | ((v[:, 128:256] & 0xFF) << 8)
                      | ((v[:, 256:384] & 0xFF) << 16) | (v[:, 384:512] << 24))
                     for v in [main] + coarse + fine]
            words.append(jnp.zeros((128 - NT * DH, 128), i32))
            wt = jnp.concatenate(words, axis=0).T
            k8_scr[h, pl.ds(pl.multiple_of(t * 128, 128), 128), :] = pltpu.bitcast(wt, u32)
            return wt[120:128]

        def body_b(t, umax):
            for b in range(TQ // QB):
                rows = half_rows(t * TQ + b * QB, QB)
                qt = _dot_nt(_upk(wT_scr[D // 2:D, :]), _upk(xn_scr[rows, :]))
                dep = functools.reduce(jnp.bitwise_or, [quant_k(t, h) for h in range(b * 8, b * 8 + 8)])
                for h in range(H):
                    q = qt[h * DH:(h + 1) * DH]
                    kmx = kmax_scr[h]
                    qa = jnp.abs(q)
                    qmx = _allred8(jnp.maximum(qa[0:8], qa[8:16]), jnp.maximum)
                    uraw = jnp.maximum(qmx * kmx * (QSCALE / (127.0 * 127.0)), 2.0 ** -60)
                    umax = jnp.maximum(umax, uraw)
                    ub = (pltpu.bitcast(uraw, i32) + 0x7FFFFF) & 0x7F800000
                    b_scr[t, h, :, b * QB:(b + 1) * QB] = ub + ((23 << 23) + (1 << 22))
                    sc = kmx * (QSCALE / 127.0) * pltpu.bitcast((254 << 23) - ub, f32)
                    sc = jnp.minimum(sc, 1e38)
                    main, fine, coarse = _limbs((q.reshape(2, 8, QB) * sc[None]).reshape(DH, QB))
                    limbs = [main] + fine + coarse + [jnp.zeros((QROWS - NT * DH, QB), i32)]
                    q8_scr[t, h, :, b * QB:(b + 1) * QB] = _pk(jnp.concatenate(limbs, axis=0).astype(i8))
                xp = _upk(_after_rows(xp_scr[rows, :], dep))
                vb = _pk(_dot_nt(_upk(wT_scr[D:3 * D // 2, :]), xp).astype(bf16))
                for h in range(H):
                    vT_scr[t, h, 0:8, b * QB:(b + 1) * QB] = vb[h * 8:(h + 1) * 8]
            return umax
        umax = lax.fori_loop(0, NQ, body_b, jnp.zeros((8, QB), f32))
        flag_ref[1] = jnp.where(jnp.max(umax) <= UNIT_MAX, 1, 0).astype(i32)

        @pl.when(flag_ref[1] == 1)
        def _():
            qm, bv, mx = fast_weights(0, 0), b_scr[0, 0], None
            for c in range(NC):
                s = fast_scores(k8_scr[0, c * CK // 4:(c + 1) * CK // 4, :], qm, bv)
                s_a[0, c * CK:(c + 1) * CK, :] = s
                cm = _tree(s, jnp.minimum)
                mx = cm if mx is None else jnp.minimum(mx, cm)
            m_scr[...] = _allred8(mx, jnp.minimum)

        @pl.when(flag_ref[1] == 0)
        def _():
            def body_s(t, carry):
                rows = half_rows(t * QB, QB)
                kk = _dot(_upk(xp_scr[rows, :]), wqkv_ref[:, D:2 * D]).astype(bf16)
                for g in range(4):
                    k_scr[g, rows, :] = _pk(kk[:, g * 128:(g + 1) * 128])
                qq = _dot_nt(_upk(wT_scr[D // 2:D, :]), _upk(xn_scr[rows, :]))
                qT_scr[t] = _pk((qq * QSCALE).astype(bf16))
                return carry
            lax.fori_loop(0, S // QB, body_s, 0)
            qm = slow_weights(0, 0)

            def body_p(c, mx):
                s = -_dot(_upk(k_scr[0, half_rows(c * CK, CK), :]), qm)
                s_a[0, pl.ds(pl.multiple_of(c * CK, CK), CK), :] = s
                return jnp.minimum(mx, _tree(s, jnp.minimum))
            mx = lax.fori_loop(0, NC, body_p, jnp.full((8, TQ), jnp.inf, f32))
            m_scr[...] = _allred8(mx, jnp.minimum)

    def next_head(h):
        hn = (h + 1) & (H - 1)
        tn = jnp.minimum(i + lax.shift_right_logical(h + 1, 5), NQ - 1)
        return hn, tn

    def probs(c, m, src, z, cols):
        n = cols.stop - cols.start
        sv = src[z, c * CK:(c + 1) * CK, cols].reshape(CK // 8, 8, n)
        return jnp.exp2(m[None] - sv).reshape(CK, n)

    def v_rows(h, c, with_ones):
        t, cc = divmod(c * CK, TQ)
        return _upk(vT_scr[t, h, 0:(16 if with_ones else 8), cc:cc + CK])

    def fast_head(h, m_cur, src, dst, z, hook=None):
        solo = hook is None
        skew, gate = (SKEW_SOLO, GATE_SOLO) if solo else (SKEW_FUSE, GATE_FUSE)
        hn, tn = next_head(h)
        qm, bv = fast_weights(tn, hn), b_scr[tn, hn]
        cols = [slice(s * HW, (s + 1) * HW) for s in range(2)]
        st = [dict(mx=None, acc=None, ss=[], m=m_cur[:, cols[s]]) for s in range(2)]

        def qk(s, c):
            kc = k8_scr[hn, c * CK // 4:(c + 1) * CK // 4, :]
            if solo and s == 1 and c >= 1:
                kc = _after_rows(kc, pltpu.bitcast(st[0]["ss"][c - 1][0:8, 0:128], i32))
            v = fast_scores(kc, qm[:, cols[s]], bv[:, cols[s]])
            dst[0, c * CK:(c + 1) * CK, cols[s]] = v
            d = st[s]
            d["ss"].append(v)
            cm = _tree(v, jnp.minimum)
            d["mx"] = cm if d["mx"] is None else jnp.minimum(d["mx"], cm)

        for c in range(skew):
            for s in range(2):
                qk(s, c)
        for c in range(NC):
            for s in range(2):
                d = st[s]
                gc, gr = divmod(c * 16 + gate, 16)
                if gc >= 0:
                    dep = d["ss"][gc][gr * 8:(gr + 1) * 8, 128:256]
                    d["m"] = _after(d["m"], jnp.concatenate([dep] * 2, axis=1))
                p = probs(c, d["m"], src, z, cols[s])
                pv = _dot(v_rows(h, c, solo), p.astype(bf16))
                pv = pv[0:24] if solo else jnp.concatenate([pv, _tree(p, jnp.add)], axis=0)
                d["acc"] = pv if d["acc"] is None else d["acc"] + pv
            for s in range(2):
                if not solo:
                    hook(2 * c + s)
                if c + skew < NC:
                    qk(s, c + skew)
        acc = jnp.concatenate([st[0]["acc"], st[1]["acc"]], axis=1)
        l = acc[16:17] if solo else jnp.sum(acc[16:24], axis=0, keepdims=True)
        oT_scr[pl.ds(pl.multiple_of(h * DH, DH), DH), :] = acc[0:16] * (1.0 / l)
        return _allred8(jnp.concatenate([st[0]["mx"], st[1]["mx"]], axis=1), jnp.minimum)

    def slow_head(h, m_cur, src, dst, z):
        hn, tn = next_head(h)
        gn = lax.shift_right_logical(hn, 3)
        qm = slow_weights(tn, hn)
        acc = lsum = mx = None
        ss = []

        def qk(c):
            nonlocal mx
            s = -_dot(_upk(k_scr[gn, c * CK // 2:(c + 1) * CK // 2, :]), qm)
            dst[0, c * CK:(c + 1) * CK, :] = s
            ss.append(s)
            cm = _tree(s, jnp.minimum)
            mx = cm if mx is None else jnp.minimum(mx, cm)

        for c in range(SKEW_SLOW):
            qk(c)
        m = m_cur
        for c in range(NC):
            if c >= 1:
                gc, gr = divmod(c * 16 + GATE_SLOW, 16)
                m = _after(m, jnp.concatenate([ss[gc][gr * 8:(gr + 1) * 8, 384:512]] * 4, axis=1))
            p = probs(c, m, src, z, slice(0, TQ))
            ls = _tree(p, jnp.add)
            lsum = ls if lsum is None else lsum + ls
            pv = _dot(v_rows(h, c, False), p.astype(bf16))
            acc = pv if acc is None else acc + pv
            if c + SKEW_SLOW < NC:
                qk(c + SKEW_SLOW)
        l = jnp.sum(lsum, axis=0, keepdims=True)
        oT_scr[pl.ds(pl.multiple_of(h * DH, DH), DH), :] = acc * (1.0 / l)
        return _allred8(mx, jnp.minimum)

    def ffn_units(j):
        rows = half_rows(j * FR, FR)
        out_rows = pl.ds(pl.multiple_of(j * FR, FR), FR)
        st = {}

        def gate_up(fc, w_ref, kh):
            ks, cs = slice(kh * 256, (kh + 1) * 256), slice(fc * 128, (fc + 1) * 128)
            r = _dot(_upk(hn_scr[rows, ks]), w_ref[ks, cs])
            if kh == 0:
                st["part"] = r
            elif w_ref is wg_ref:
                st["g"] = r + st.pop("part")
            else:
                g, u = st.pop("g"), r + st.pop("part")
                a = g * u * (0.5 * jnp.tanh(0.5 * g) + 0.5)
                a_scr[:, cs] = _pk(a.astype(bf16))

        def down(oc, kh):
            ks, cs = slice(kh * 256, (kh + 1) * 256), slice(oc * 128, (oc + 1) * 128)
            y = _dot(_upk(a_scr[:, ks]), wd_ref[ks, cs])
            if kh > 0:
                y = y + st.pop("y")
            if kh < F // 256 - 1:
                st["y"] = y
            else:
                o_ref[out_rows, cs] = (h1_scr[out_rows, cs] + y).astype(o_ref.dtype)

        units = [functools.partial(gate_up, fc, w_ref, kh)
                 for fc in range(F // 128) for w_ref in (wg_ref, wu_ref) for kh in range(2)]
        units += [functools.partial(down, oc, kh) for oc in range(4) for kh in range(F // 256)]
        return units

    def heads_loop(head_fn, unroll, with_ffn=False):
        def body(j, m):
            z = flag_ref[0]
            slots = {}
            if with_ffn:
                units = ffn_units(j)
                for n, fn in enumerate(units):
                    step = int(2 + n / len(units) * (unroll * NC - 4))
                    slots.setdefault(2 * step + n % 2, []).append(fn)
            for u in range(unroll):
                src, dst = (s_a, s_b) if u % 2 == 0 else (s_b, s_a)
                args = (j * unroll + u, m, src, dst, z)
                if with_ffn:
                    def hook(pos, u=u):
                        for fn in slots.get(u * NC * 2 + pos, []):
                            fn()
                    m = head_fn(*args, hook)
                else:
                    m = head_fn(*args)
            return m
        m_scr[...] = lax.fori_loop(0, H // unroll, body, m_scr[...])

    fast = flag_ref[1] == 1

    @pl.when(i == 1)
    def _():
        for j in range(1, 4):
            w_copy(j).wait()

    @pl.when(jnp.logical_and(fast, i == 0))
    def _():
        heads_loop(fast_head, UNR_FAST)

    @pl.when(jnp.logical_and(fast, jnp.logical_and(i > 0, i < NQ)))
    def _():
        heads_loop(fast_head, UNR_FAST, with_ffn=True)

    @pl.when(jnp.logical_or(i == NQ, jnp.logical_and(i > 0, jnp.logical_not(fast))))
    def _():
        def ffn_body(j, carry):
            for fn in ffn_units(j):
                fn()
            return carry
        lax.fori_loop(0, TQ // FR, ffn_body, 0)

    @pl.when(jnp.logical_and(jnp.logical_not(fast), i < NQ))
    def _():
        heads_loop(slow_head, UNR_SLOW)

    @pl.when(i == 0)
    def _():
        w_copy(0).wait()

    @pl.when(i < NQ)
    def _():
        for b in range(TQ // FR):
            r0 = pl.multiple_of(i * TQ + b * FR, FR)
            o = oT_scr[:, b * FR:(b + 1) * FR].T.astype(bf16)
            h1 = x_ref[pl.ds(r0, FR), :].astype(f32) + _dot(o, wo_ref[...])
            h1_scr[b * FR:(b + 1) * FR, :] = h1
            hn_scr[b * FR // 2:(b + 1) * FR // 2, :] = _pk(_ln(h1).astype(bf16))


@jax.jit
def pallas_sequential_preLN__softmax_full_mha__swiglu_ffn__prompt_kernel(
    A_x: jax.Array,
    A_wqkv: jax.Array,
    A_wo: jax.Array,
    B_x: jax.Array,
    B_w_gate: jax.Array,
    B_w_up: jax.Array,
    B_w_down: jax.Array,
):
    del B_x
    out = pl.pallas_call(
        _kernel,
        grid=(NQ + 1,),
        in_specs=[pl.BlockSpec(memory_space=pl.ANY)] * 6,
        out_specs=pl.BlockSpec((TQ, D), lambda i: (jnp.maximum(i - 1, 0), 0)),
        out_shape=jax.ShapeDtypeStruct((S, D), bf16),
        scratch_shapes=[
            pltpu.VMEM((S, D), bf16),
            pltpu.VMEM((D, 3 * D), bf16),
            pltpu.VMEM((D, D), bf16),
            pltpu.VMEM((D, F), bf16),
            pltpu.VMEM((D, F), bf16),
            pltpu.VMEM((F, D), bf16),
            pltpu.SemaphoreType.DMA((NQ + 7,)),
            pltpu.VMEM((3 * D // 2, D), u32),
            pltpu.VMEM((S // 2, D), u32),
            pltpu.VMEM((S // 2, D), u32),
            pltpu.VMEM((2, 4, TQ, 128), f32),
            pltpu.VMEM((NQ, D, TQ), f32),
            pltpu.VMEM((H, 8, 128), f32),
            pltpu.VMEM((H, S // 4, 128), u32),
            pltpu.VMEM((NQ, H, QROWS // 4, TQ), u32),
            pltpu.VMEM((NQ, H, 8, TQ), i32),
            pltpu.VMEM((NQ, H, 16, TQ), u32),
            pltpu.VMEM((4, S // 2, 128), u32),
            pltpu.VMEM((S // QB, D // 2, QB), u32),
            pltpu.VMEM((1, S, TQ), f32),
            pltpu.VMEM((1, S, TQ), f32),
            pltpu.VMEM((8, TQ), f32),
            pltpu.VMEM((D, TQ), f32),
            pltpu.VMEM((TQ, D), f32),
            pltpu.VMEM((TQ // 2, D), u32),
            pltpu.VMEM((FR // 2, F), u32),
            pltpu.SMEM((2,), i32),
        ],
        compiler_params=pltpu.CompilerParams(
            dimension_semantics=("arbitrary",),
            vmem_limit_bytes=110 * 1024 * 1024,
        ),
    )(A_x.reshape(S, D), A_wqkv, A_wo, B_w_gate, B_w_up, B_w_down)
    return out.reshape(1, S, D)
```
